```python
import os as _os
_os.environ.setdefault("JAX_PLATFORMS", "cpu")
import jax
import jax.numpy as jnp

def _softmax(x, axis=-1):
    return jax.nn.softmax(x, axis=axis)
def _gelu(x):
    return jax.nn.gelu(x, approximate=True)
def _silu(x):
    return jax.nn.silu(x)
def _sigmoid(x):
    return jax.nn.sigmoid(x)
def _layernorm(x, axis=-1, eps=1e-5):
    m = jnp.mean(x, axis=axis, keepdims=True)
    v = jnp.var(x, axis=axis, keepdims=True)
    return (x - m) / jnp.sqrt(v + eps)
def _scatter_add(tgt, idx, src, axis=0):
    return tgt.at[idx].add(src)
def _segment_sum(src, seg, n):
    return jax.ops.segment_sum(src, seg, n)
class _Rng:
    def __init__(self, key):
        self._k = key
    def _next(self):
        self._k, sub = jax.random.split(self._k)
        return sub
    def normal(self, shape):
        return jax.random.normal(self._next(), shape, dtype=jnp.bfloat16)
    def randint(self, lo, hi, shape):
        return jax.random.randint(self._next(), shape, lo, hi, dtype=jnp.int32)
    def uniform(self, shape, lo=0.0, hi=1.0):
        return jax.random.uniform(self._next(), shape, jnp.bfloat16, lo, hi)
    def permutation(self, n):
        return jax.random.permutation(self._next(), n)


kernel_name = 'concat_heads__spectral_gfnet__sliding_block__prompt'

def setup_inputs():
    _rng = _Rng(jax.random.key(int.from_bytes(__import__("os").urandom(4), "little")))
    _w = (lambda a: (lambda t: t.astype(jnp.bfloat16) if jnp.issubdtype(t.dtype, jnp.floating) else t)(jnp.asarray(a)))
    def _A_setup():
        B, S, D = 1, 2048, 640
        Df = D // 2 + 1
        return {
            "x": _w((lambda *s: _rng.normal(s) * 0.05)(B, S, D)),
            "w_r": _w((lambda *s: _rng.normal(s) * 0.4)(S, Df) * 0.02),
            "w_i": _w((lambda *s: _rng.normal(s) * 0.4)(S, Df) * 0.02),
        }
    _A_in = _A_setup()

    def _B_setup():
        B, S, D = 1, 2048, 640
        return {
            "x": _w((lambda *s: _rng.normal(s) * 0.2)(B, S, D)),
            "wqkv": _w((lambda *s: _rng.normal(s) * 0.2)(D, 3 * D)),
            "wo": _w((lambda *s: _rng.normal(s) * 0.05)(D, D)),
        }
    _B_in = _B_setup()

    return {
        "A_x": _A_in["x"],
        "A_w_r": _A_in["w_r"],
        "A_w_i": _A_in["w_i"],
        "B_x": _B_in["x"],
        "B_wqkv": _B_in["wqkv"],
        "B_wo": _B_in["wo"],
    }

def reference(A_x, A_w_r, A_w_i, B_x, B_wqkv, B_wo):
    def _A_ref(x, w_r, w_i):
        B, S, D = x.shape
        X = (lambda x, axes=(-2,-1): jnp.fft.rfft2(x.astype(jnp.float32), axes=axes))(x, axes=(-2, -1))
        W = w_r + 1j * w_i
        X = X * W
        y = (lambda x, s, axes=(-2,-1): jnp.fft.irfft2(x, s=s, axes=axes).astype(jnp.bfloat16))(X, (S, D), axes=(-2, -1))
        return y

    def _B_ref(x, wqkv, wo):
        B, S, D = x.shape
        H = 32; Dh = D // H; W = 256
        qkv = (lambda x, *d: x.transpose(*d))((x @ wqkv).reshape(B, S, 3, H, Dh), 2, 0, 3, 1, 4)
        q, k, v = qkv[0], qkv[1], qkv[2]
        scores = jnp.einsum("bhqd,bhkd->bhqk", q, k) * (Dh ** -0.5)
        idx = jnp.arange(S)
        mask = (idx[:, None] - idx[None, :] >= 0) & (idx[:, None] - idx[None, :] < W)
        scores = jnp.where(mask[None, None], scores, -1e9)
        p = _softmax(scores, axis=-1)
        o = jnp.einsum("bhqk,bhkd->bhqd", p, v)
        return (lambda x, *d: x.transpose(*d))(o, 0, 2, 1, 3).reshape(B, S, D) @ wo

    a = _A_ref(A_x, A_w_r, A_w_i)
    b = _B_ref(B_x, B_wqkv, B_wo)
    return jnp.concatenate([a, b], axis=-1)
```

```python
import functools
import math

import jax
import jax.numpy as jnp
import numpy as np
import ml_dtypes
from jax.experimental import pallas as pl
from jax.experimental.pallas import tpu as pltpu

S = 2048
D = 640
DF = 321
H = 32
DH = 20
NB = 16
NEG = -1e30
SCALE = (DH ** -0.5) * 1.4426950408889634
bf16 = jnp.bfloat16
f32 = jnp.float32
u32 = jnp.uint32
i32 = jnp.int32
NT = (((1,), (1,)), ((), ()))
C1, C2 = math.cos(2 * math.pi / 5), math.cos(4 * math.pi / 5)
S1, S2 = math.sin(2 * math.pi / 5), math.sin(4 * math.pi / 5)


def _make_consts():
    l = np.arange(128)
    k1 = np.where(l < 64, 1 + 5 * l, 4 + 5 * (l - 64))
    k2 = np.where(l < 64, 2 + 5 * l, 3 + 5 * (l - 64))
    k0 = np.where(l <= 64, 5 * l, 0)
    n = np.arange(128)[:, None]
    sig = np.where(l < 64, 1.0, -1.0)[None, :]

    def cs(k):
        th = 2 * np.pi * ((n * k[None, :]) % D) / D
        return np.cos(th), np.sin(th)

    ms = []
    for k in (k1, k2):
        c, s = cs(k)
        ms.append(np.block([[c, -s], [sig * s, sig * c]]))
    c, s = cs(k0)
    v = (l <= 64)[None, :]
    m0 = np.concatenate([c * v, -s * v], axis=1)
    ck0 = np.where((k0 == 0) | (k0 == 320), 1.0, 2.0) * (l <= 64)
    n0 = (m0 * np.concatenate([ck0, ck0])[None, :]).T / (S * D)
    mf = np.concatenate([ms[0], ms[1], m0], axis=0)
    nf = np.concatenate([ms[0].T * (2.0 / (S * D)), ms[1].T * (2.0 / (S * D)), n0], axis=1)
    a1 = np.arange(32)[:, None, None]
    a2 = np.arange(64)[None, :, None]
    n2 = np.arange(64)[None, None, :]
    a = 2 * np.pi * ((n2 * (a1 + 32 * a2)) % S) / S
    gr, gi = np.cos(a), -np.sin(a)
    g = np.concatenate([np.concatenate([gr, -gi], axis=2), np.concatenate([gi, gr], axis=2)], axis=1)
    hm = np.transpose(g, (0, 2, 1))
    cvt = lambda z: np.ascontiguousarray(z).astype(ml_dtypes.bfloat16)
    return cvt(mf), cvt(nf), cvt(g), cvt(hm)


def pk(x):
    return pltpu.bitcast(x, u32)


def unpk(x):
    return pltpu.bitcast(x, bf16)


def _cmul(re, im, wr, wi):
    e = 1e-12
    if abs(wi) < e:
        if abs(wr - 1) < e:
            return re, im
        return re * wr, im * wr
    if abs(abs(wr) - abs(wi)) < e:
        if wi / wr > 0:
            return (re - im) * wr, (re + im) * wr
        return (re + im) * wr, (im - re) * wr
    return re * wr - im * wi, re * wi + im * wr


def _fft(xr, xi, sgn):
    n = len(xr)
    if n == 1:
        return xr, xi
    if n == 2:
        return [xr[0] + xr[1], xr[0] - xr[1]], [xi[0] + xi[1], xi[0] - xi[1]]
    er, ei = _fft(xr[0::2], xi[0::2], sgn)
    ar, ai = _fft(xr[1::4], xi[1::4], sgn)
    br, bi = _fft(xr[3::4], xi[3::4], sgn)
    outr = [None] * n
    outi = [None] * n
    q = n // 4
    for k in range(q):
        a1 = sgn * 2 * math.pi * k / n
        a3 = 3 * a1
        z1r, z1i = _cmul(ar[k], ai[k], math.cos(a1), math.sin(a1))
        z3r, z3i = _cmul(br[k], bi[k], math.cos(a3), math.sin(a3))
        sr, si = z1r + z3r, z1i + z3i
        dr, di = z1r - z3r, z1i - z3i
        outr[k], outi[k] = er[k] + sr, ei[k] + si
        outr[k + 2 * q], outi[k + 2 * q] = er[k] - sr, ei[k] - si
        if sgn < 0:
            outr[k + q], outi[k + q] = er[k + q] + di, ei[k + q] - dr
            outr[k + 3 * q], outi[k + 3 * q] = er[k + q] - di, ei[k + q] + dr
        else:
            outr[k + q], outi[k + q] = er[k + q] - di, ei[k + q] + dr
            outr[k + 3 * q], outi[k + 3 * q] = er[k + q] + di, ei[k + q] - dr
    return outr, outi


def _dot(a, b):
    return jnp.dot(a, b, preferred_element_type=f32)


def _kernel(xa_h, wrT_h, wiT_h, xb_h, wqkv_h, wo_h, mf_h, nf_h, g_h, h_h, out_h,
            xa_v, wrT_v, wiT_v, xb_v, wqkv_v, wo_v, mf_v, nf_v, g_v, h_v, oa_v, ob_v,
            mf_s, nf_s, u_s, st_s, wp_s,
            wqvT_s, wk_s, wo_s, bias_s, z_s, wq_s, vw_s, kw_s, o_s,
            isem, osem):
    def cp(src, dst, k):
        return pltpu.make_async_copy(src, dst, isem.at[k])

    def rows(ref, c, n):
        return ref.at[pl.ds(c * n, n), :]

    d_mf = cp(mf_h, mf_v, 0)
    d_xa = [cp(rows(xa_h, c, 512), rows(xa_v, c, 512), 1 + c) for c in range(4)]
    d_wk = cp(wqkv_h.at[:, D:2 * D], wqkv_v.at[:, D:2 * D], 5)
    d_xb = [cp(rows(xb_h, c, 512), rows(xb_v, c, 512), 6 + c) for c in range(4)]
    d_wq = cp(wqkv_h.at[:, 0:D], wqkv_v.at[:, 0:D], 10)
    d_wv = cp(wqkv_h.at[:, 2 * D:3 * D], wqkv_v.at[:, 2 * D:3 * D], 11)
    d_wr = cp(wrT_h, wrT_v, 12)
    d_wi = cp(wiT_h, wiT_v, 13)
    d_g = cp(g_h, g_v, 14)
    d_h = cp(h_h, h_v, 15)
    d_wo = cp(wo_h, wo_v, 16)
    d_nf = cp(nf_h, nf_v, 17)

    d_mf.start()
    d_xa[0].start()
    d_xa[1].start()

    def p1_block(i):
        r0 = pl.multiple_of(i * 128, 128)
        xt = [xa_v[pl.ds(r0, 128), t * 128:(t + 1) * 128].astype(f32) for t in range(5)]
        t1, t2 = xt[1] + xt[4], xt[2] + xt[3]
        t3, t4 = xt[1] - xt[4], xt[2] - xt[3]
        y0 = (xt[0] + t1 + t2).astype(bf16)
        y1r = (xt[0] + C1 * t1 + C2 * t2).astype(bf16)
        y2r = (xt[0] + C2 * t1 + C1 * t2).astype(bf16)
        y1i = ((-S1) * t3 - S2 * t4).astype(bf16)
        y2i = ((-S2) * t3 + S1 * t4).astype(bf16)
        for p, (yr, yi) in enumerate(((y1r, y1i), (y2r, y2i))):
            for n in range(2):
                m_r = unpk(mf_s[p * 128:p * 128 + 64, n * 128:(n + 1) * 128])
                m_i = unpk(mf_s[p * 128 + 64:p * 128 + 128, n * 128:(n + 1) * 128])
                u_s[p + 3 * n, pl.ds(r0, 128), :] = _dot(yr, m_r) + _dot(yi, m_i)
        for n in range(2):
            u_s[2 + 3 * n, pl.ds(r0, 128), :] = _dot(y0, unpk(mf_s[256:320, n * 128:(n + 1) * 128]))

    def fft_set(p, r, sgn):
        off = pl.multiple_of(r * 8, 8)
        xr = [u_s[p, pl.ds(64 * n + off, 8), :] for n in range(32)]
        xi = [u_s[3 + p, pl.ds(64 * n + off, 8), :] for n in range(32)]
        yr, yi = _fft(xr, xi, sgn)
        for n in range(32):
            u_s[p, pl.ds(64 * n + off, 8), :] = yr[n]
            u_s[3 + p, pl.ds(64 * n + off, 8), :] = yi[n]

    def wprep(T):
        c0 = pl.multiple_of(T * 128, 128)
        q0 = pl.multiple_of(T * 64, 64)
        zer = jnp.zeros((56, 128), f32)
        sub = jax.lax.broadcasted_iota(i32, (8, 128), 0)
        for j, ref in enumerate((wrT_v, wiT_v)):
            st_s[j, 0:320, :] = ref[0:320, pl.ds(c0, 128)].astype(f32)
            last = jnp.broadcast_to(ref[320:321, pl.ds(c0, 128)].astype(f32), (8, 128))
            last = jnp.where(sub == 0, last, 0.0)
            sl = lambda a: st_s[j, pl.ds(a, 64, stride=5), :]
            tiles = (jnp.concatenate([sl(1), sl(4)], axis=0),
                     jnp.concatenate([sl(2), sl(3)], axis=0),
                     jnp.concatenate([sl(0), last, zer], axis=0))
            for p in range(3):
                wp_s[3 * j + p, pl.ds(q0, 64), :] = pk(tiles[p].astype(bf16).T)

    def mid_pair(a):
        wv = [wp_s[t, pl.ds(a, 64, stride=16), :] for t in range(6)]
        for j in range(2):
            k1 = 2 * a + j
            r0 = pl.multiple_of(k1 * 64, 64)
            if j == 0:
                wf = [pltpu.bitcast(w << 16, f32) for w in wv]
            else:
                wf = [pltpu.bitcast(w & jnp.uint32(0xFFFF0000), f32) for w in wv]
            gk, hk = g_v[k1], h_v[k1]
            for p in range(3):
                y = jnp.concatenate([u_s[p, pl.ds(r0, 64), :], u_s[3 + p, pl.ds(r0, 64), :]], axis=0).astype(bf16)
                x = _dot(gk, y)
                xr, xi = x[0:64], x[64:128]
                wr, wi = wf[p], wf[3 + p]
                pp = jnp.concatenate([xr * wr - xi * wi, xr * wi + xi * wr], axis=0).astype(bf16)
                z = _dot(hk, pp)
                u_s[p, pl.ds(r0, 64), :] = z[0:64]
                u_s[3 + p, pl.ds(r0, 64), :] = z[64:128]

    def p5_block(i):
        r0 = pl.multiple_of(i * 128, 128)
        z = [u_s[t, pl.ds(r0, 128), :].astype(bf16) for t in range(6)]

        def prod(p, c0):
            return (_dot(z[p], unpk(nf_s[0:64, c0:c0 + 128])) + _dot(z[3 + p], unpk(nf_s[64:128, c0:c0 + 128])))
        r1, i1 = prod(0, 0), prod(0, 128)
        r2, i2 = prod(1, 256), prod(1, 384)
        t0 = prod(2, 512)
        a1 = t0 + C1 * r1 + C2 * r2
        b1 = S1 * i1 + S2 * i2
        a2 = t0 + C2 * r1 + C1 * r2
        b2 = S2 * i1 - S1 * i2
        ys = (t0 + r1 + r2, a1 - b1, a2 - b2, a2 + b2, a1 + b1)
        for t in range(5):
            oa_v[pl.ds(r0, 128), t * 128:(t + 1) * 128] = ys[t].astype(bf16)
        pltpu.make_async_copy(oa_v.at[pl.ds(r0, 128), :], out_h.at[pl.ds(r0, 128), 0:D], osem.at[0, i]).start()

    def setup_misc():
        row = jax.lax.broadcasted_iota(i32, (128, 128), 0)
        lane = jax.lax.broadcasted_iota(i32, (128, 128), 1)
        bias_s[0] = jnp.where(row > lane, 0.0, NEG).astype(f32)
        bias_s[1] = jnp.zeros((128, 128), f32)
        bias_s[2] = jnp.where(row <= lane, 0.0, NEG).astype(f32)
        z_s[...] = jnp.zeros(z_s.shape, i32)

    def setup_qv():
        for part, c0 in ((0, 0), (1, 2 * D)):
            for n in range(5):
                for kt in range(5):
                    t = wqkv_v[kt * 128:(kt + 1) * 128, c0 + n * 128:c0 + (n + 1) * 128].T
                    wqvT_s[part * 320 + n * 64:part * 320 + (n + 1) * 64, kt * 128:(kt + 1) * 128] = pk(t)

    def proj_k(i):
        r0 = pl.multiple_of(i * 128, 128)
        xi = xb_v[pl.ds(r0, 128), :]
        tiles = []
        for n in range(5):
            acc = None
            for kt in range(5):
                r = _dot(xi[:, kt * 128:(kt + 1) * 128], unpk(wk_s[kt * 64:(kt + 1) * 64, n * 128:(n + 1) * 128]))
                acc = r if acc is None else acc + r
            tiles.append(pk(acc.astype(bf16)))
        lane = jax.lax.broadcasted_iota(i32, (64, 128), 1)
        for g in range(8):
            off = (80 * g) % 128
            ta = (80 * g) // 128
            if off == 0:
                w = tiles[ta]
            else:
                w = pltpu.roll(tiles[ta], 128 - off, 1)
                if off + 80 > 128:
                    w = jnp.where(lane < 128 - off, w, pltpu.roll(tiles[ta + 1], 128 - off, 1))
            kw_s[i, :, g * 128:(g + 1) * 128] = w

    def proj_qv(i):
        r0_ = pl.multiple_of(i * 128, 128)
        xi = xb_v[pl.ds(r0_, 128), :]

        def chunks(part):
            outs = []
            for c in range(2):
                acc = None
                for kt in range(5):
                    lhs = unpk(wqvT_s[part * 320 + c * 160:part * 320 + (c + 1) * 160, kt * 128:(kt + 1) * 128])
                    r = jax.lax.dot_general(lhs, xi[:, kt * 128:(kt + 1) * 128], NT, preferred_element_type=f32)
                    acc = r if acc is None else acc + r
                outs.append(acc)
            return jnp.concatenate(outs, axis=0)
        row = jax.lax.broadcasted_iota(i32, (32, 128), 0)
        qT = chunks(0) * SCALE
        for h in range(H):
            r0 = (20 * h) // 16 * 16
            dl = 20 * h - r0
            w = jnp.where((row >= dl) & (row < dl + 20), qT[r0:r0 + 32], 0.0)
            wq_s[i, h] = pk(w.astype(bf16))
        vT = chunks(1)
        ones = jnp.ones((8, 128), f32)
        for h in range(H):
            r0 = (20 * h) // 16 * 16
            dl = 20 * h - r0
            if dl <= 4:
                w = jnp.concatenate([vT[r0:r0 + 24], ones], axis=0)
            else:
                w = jnp.concatenate([ones, vT[r0 + 8:r0 + 32]], axis=0)
            vw_s[i, h] = pk(w.astype(bf16))

    def out_proj(i):
        r0 = pl.multiple_of(i * 128, 128)
        ot = [unpk(o_s[:, n * 128:(n + 1) * 128]) for n in range(5)]
        for n in range(5):
            acc = None
            for kt in range(5):
                r = _dot(ot[kt], unpk(wo_s[kt * 64:(kt + 1) * 64, n * 128:(n + 1) * 128]))
                acc = r if acc is None else acc + r
            ob_v[pl.ds(r0, 128), n * 128:(n + 1) * 128] = acc.astype(bf16)
        pltpu.make_async_copy(ob_v.at[pl.ds(r0, 128), :], out_h.at[pl.ds(r0, 128), D:2 * D], osem.at[1, i]).start()

    def attention(i, lag=4):
        zero = z_s[...]

        def getw(g, h):
            o = 20 * h - 80 * g
            r0 = o // 16 * 16
            parts = []
            if r0 > 0:
                parts.append(jnp.zeros((r0, 128), bf16))
            parts.append(unpk(wq_s[i, h]))
            if 96 - r0 > 0:
                parts.append(jnp.zeros((96 - r0, 128), bf16))
            return jnp.concatenate(parts, axis=0)
        kb = [jnp.maximum(i - 2 + t, 0) for t in range(3)]
        allneg = jnp.full((128, 128), NEG, f32)
        bias = [jnp.where(i >= 2, bias_s[0], allneg), jnp.where(i >= 1, bias_s[1], allneg), bias_s[2]]
        sv, mx, acc, tok, res = {}, {}, {}, {}, {}

        def qk(k):
            g, t = divmod(k, 3)
            kk = unpk(kw_s[kb[t], :, g * 128:(g + 1) * 128])
            for j, h in enumerate(range(4 * g, 4 * g + 4)):
                st = _dot(kk, getw(g, h))
                tok[(k, j)] = pltpu.bitcast(st[0:8], i32) & zero
                st = st + bias[t]
                sv[(k, j)] = st
                mm = jnp.max(st.reshape(16, 8, 128), axis=0)
                mx[h] = mm if t == 0 else jnp.maximum(mx[h], mm)
                if t == 2:
                    mx[h] = jnp.broadcast_to(jnp.max(mx[h], axis=0, keepdims=True), (8, 128))

        def pv(k, kt):
            g, t = divmod(k, 3)
            for j, h in enumerate(range(4 * g, 4 * g + 4)):
                m = mx[h]
                if kt is not None:
                    m = pltpu.bitcast(pltpu.bitcast(m, i32) | tok[(kt, j)], f32)
                s = sv.pop((k, j))
                p = jnp.exp2(s.reshape(16, 8, 128) - m[None]).reshape(128, 128).astype(bf16)
                r = _dot(unpk(vw_s[kb[t], h]), p)
                acc[h] = r if t == 0 else acc[h] + r
                if t == 2:
                    r0 = (20 * h) // 16 * 16
                    dl = 20 * h - r0
                    l = acc[h][24:32] if dl <= 4 else acc[h][0:8]
                    res[h] = (acc[h].reshape(4, 8, 128) * (1.0 / l)[None]).reshape(32, 128)
        nk = 24
        for k in range(nk + lag):
            if k < nk:
                qk(k)
            if k - lag >= 0:
                kt = k - 1
                if kt >= nk or kt < 0:
                    kt = None
                pv(k - lag, kt)
        sub = jax.lax.broadcasted_iota(i32, (8, 128), 0)
        vregs = []
        for v in range(80):
            h0, h1 = (8 * v) // 20, (8 * v + 7) // 20

            def get(h):
                r0 = (20 * h) // 16 * 16
                return res[h][8 * v - r0:8 * v - r0 + 8]
            vregs.append(get(h0) if h0 == h1 else jnp.where(sub < (20 * h1 - 8 * v), get(h0), get(h1)))
        oT = jnp.concatenate(vregs, axis=0).astype(bf16)
        for n in range(5):
            o_s[:, n * 128:(n + 1) * 128] = pk(oT[n * 128:(n + 1) * 128].T)

    setup_misc()
    st_s[0, 320:328, :] = jnp.zeros((8, 128), f32)
    st_s[1, 320:328, :] = jnp.zeros((8, 128), f32)
    d_mf.wait()
    mf_s[...] = pk(mf_v[...])

    def loop_a(c, carry):
        @pl.when(c == 0)
        def _():
            d_xa[0].wait()
            d_xa[2].start()

        @pl.when(c == 1)
        def _():
            d_xa[1].wait()
            d_xa[3].start()

        @pl.when(c == 2)
        def _():
            d_xa[2].wait()
            d_wk.start()
            d_xb[0].start()

        @pl.when(c == 3)
        def _():
            d_xa[3].wait()
            d_xb[1].start()
            d_wq.start()
            d_wv.start()
        for j in range(4):
            p1_block(4 * c + j)
        return carry
    jax.lax.fori_loop(0, 4, loop_a, 0)

    d_wk.wait()
    wk_s[...] = pk(wqkv_v[:, D:2 * D])

    def loop_b(it, carry):
        @pl.when(it == 0)
        def _():
            d_xb[0].wait()
            d_xb[2].start()
            d_wr.start()
            d_wi.start()

        @pl.when(it == 2)
        def _():
            d_xb[1].wait()
            d_xb[3].start()

        @pl.when(it == 4)
        def _():
            d_xb[2].wait()
            d_wr.wait()
            d_wi.wait()
            d_g.start()
            d_h.start()

        @pl.when(it == 6)
        def _():
            d_xb[3].wait()
            d_wo.start()
            d_nf.start()
        proj_k(2 * it)
        proj_k(2 * it + 1)
        for j in range(3):
            fft_set(j, it, -1)
        return carry
    jax.lax.fori_loop(0, 8, loop_b, 0)

    d_wq.wait()
    d_wv.wait()
    setup_qv()

    def loop_w(T, carry):
        wprep(T)
        return carry
    jax.lax.fori_loop(0, 16, loop_w, 0)

    d_g.wait()
    d_h.wait()

    def loop_c(it, carry):
        proj_qv(it)
        mid_pair(2 * it)
        mid_pair(2 * it + 1)
        return carry
    jax.lax.fori_loop(0, 8, loop_c, 0)

    d_wo.wait()
    d_nf.wait()
    wo_s[...] = pk(wo_v[...])
    nf_s[...] = pk(nf_v[...])

    def loop_d(it, carry):
        proj_qv(8 + it)
        for j in range(3):
            fft_set(j, it, +1)
        return carry
    jax.lax.fori_loop(0, 8, loop_d, 0)

    o_s[...] = jnp.zeros(o_s.shape, u32)

    def loop_e(i, carry):
        p5_block(i)
        attention(i)
        out_proj(i)
        return carry
    jax.lax.fori_loop(0, NB, loop_e, 0)

    def loop_f(i, carry):
        r0 = pl.multiple_of(i * 128, 128)
        pltpu.make_async_copy(oa_v.at[pl.ds(r0, 128), :], out_h.at[pl.ds(r0, 128), 0:D], osem.at[0, i]).wait()
        pltpu.make_async_copy(ob_v.at[pl.ds(r0, 128), :], out_h.at[pl.ds(r0, 128), D:2 * D], osem.at[1, i]).wait()
        return carry
    jax.lax.fori_loop(0, NB, loop_f, 0)


_CONSTS = _make_consts()


@jax.jit
def pallas_concat_heads__spectral_gfnet__sliding_block__prompt_kernel(A_x, A_w_r, A_w_i, B_x, B_wqkv, B_wo):
    mf, nf, g, hm = _CONSTS
    vm = pltpu.VMEM
    out = pl.pallas_call(
        _kernel,
        out_shape=jax.ShapeDtypeStruct((S, 2 * D), bf16),
        in_specs=[pl.BlockSpec(memory_space=pl.ANY)] * 10,
        out_specs=pl.BlockSpec(memory_space=pl.ANY),
        scratch_shapes=[
            vm((S, D), bf16), vm((DF, S), bf16), vm((DF, S), bf16), vm((S, D), bf16), vm((D, 3 * D), bf16),
            vm((D, D), bf16), vm((640, 256), bf16), vm((256, 640), bf16), vm((32, 128, 128), bf16),
            vm((32, 128, 128), bf16), vm((S, D), bf16), vm((S, D), bf16),
            vm((320, 256), u32), vm((128, 640), u32), vm((6, S, 128), f32), vm((2, 328, 128), f32),
            vm((6, 1024, 128), u32),
            vm((640, 640), u32), vm((320, 640), u32), vm((320, 640), u32), vm((3, 128, 128), f32),
            vm((8, 128), i32), vm((NB, H, 16, 128), u32), vm((NB, H, 16, 128), u32), vm((NB, 64, 1024), u32),
            vm((64, 640), u32),
            pltpu.SemaphoreType.DMA((18,)), pltpu.SemaphoreType.DMA((2, NB)),
        ],
        compiler_params=pltpu.CompilerParams(vmem_limit_bytes=120 * 1024 * 1024),
        name="fused_kernel",
    )(A_x.reshape(S, D), A_w_r.T, A_w_i.T, B_x.reshape(S, D), B_wqkv, B_wo, mf, nf, g, hm)
    return out.reshape(1, S, 2 * D)
```

```python
import functools
import math

import jax
import jax.numpy as jnp
import numpy as np
import ml_dtypes
from jax.experimental import pallas as pl
from jax.experimental.pallas import tpu as pltpu

CFG = dict(
    xb_split=(256, 768), a_mode="line", b_mode="line", b_late=-1, late_mid=True, a_conv=16, w_early=True, k_loop=1, g4=True, kc_gate=0, dkeys=(0, 2, 3, 4, 5, 5, 5), c_mode=2, d_mode="line",
    fft_tok=3, lag=5, tokoff=1, dtok=1, p5_pre=0, p5b_pre=None, drain='ladder6', rcp_newton=True, pad=0, e_un=2, st_dbl=True, k_first=256,
)
S = 2048
D = 640
DF = 321
H = 32
DH = 20
NB = 16
NEG = -1e30
SCALE = (DH ** -0.5) * 1.4426950408889634
bf16 = jnp.bfloat16
f32 = jnp.float32
u32 = jnp.uint32
i32 = jnp.int32
NT = (((1,), (1,)), ((), ()))
C1, C2 = math.cos(2 * math.pi / 5), math.cos(4 * math.pi / 5)
S1, S2 = math.sin(2 * math.pi / 5), math.sin(4 * math.pi / 5)


def _make_consts():
    l = np.arange(128)
    k1 = np.where(l < 64, 1 + 5 * l, 4 + 5 * (l - 64))
    k2 = np.where(l < 64, 2 + 5 * l, 3 + 5 * (l - 64))
    n = np.arange(128)[:, None]
    sig = np.where(l < 64, 1.0, -1.0)[None, :]

    def cs(k):
        th = 2 * np.pi * ((n * k[None, :]) % D) / D
        return np.cos(th), np.sin(th)

    ms = []
    for k in (k1, k2):
        c, s = cs(k)
        ms.append(np.block([[c, -s], [sig * s, sig * c]]))
    k0 = np.where(l <= 64, 5 * l, 5 * (l - 64))
    c, s = cs(k0)
    low = (l <= 64)[None, :]
    m0 = np.where(low, c, -s)
    ck0 = np.where((k0 == 0) | (k0 == 320), 1.0, 2.0)
    n0 = (m0 * ck0[None, :]).T / (S * D)
    mf = np.concatenate([np.concatenate(ms, axis=0),
                         np.concatenate([m0, np.zeros((128, 128))], axis=1)], axis=0)
    nf = np.concatenate([ms[0].T * (2.0 / (S * D)), ms[1].T * (2.0 / (S * D)),
                         np.concatenate([n0, np.zeros((128, 128))], axis=0)], axis=1)
    a1 = np.arange(32)[:, None, None]
    a2 = np.arange(64)[None, :, None]
    n2 = np.arange(64)[None, None, :]
    a = 2 * np.pi * ((n2 * (a1 + 32 * a2)) % S) / S
    gr, gi = np.cos(a), -np.sin(a)
    g = np.concatenate([np.concatenate([gr, -gi], axis=2), np.concatenate([gi, gr], axis=2)], axis=1)
    hm = np.transpose(g, (0, 2, 1))
    cvt = lambda z: np.ascontiguousarray(z).astype(ml_dtypes.bfloat16)
    return cvt(mf), cvt(nf), cvt(g), cvt(hm)


def pk(x):
    return pltpu.bitcast(x, u32)


def unpk(x):
    return pltpu.bitcast(x, bf16)


def _cmul(re, im, wr, wi):
    e = 1e-12
    if abs(wi) < e:
        if abs(wr - 1) < e:
            return re, im
        return re * wr, im * wr
    if abs(abs(wr) - abs(wi)) < e:
        if wi / wr > 0:
            return (re - im) * wr, (re + im) * wr
        return (re + im) * wr, (im - re) * wr
    return re * wr - im * wi, re * wi + im * wr


def _fft(xr, xi, sgn):
    n = len(xr)
    if n == 1:
        return xr, xi
    if n == 2:
        return [xr[0] + xr[1], xr[0] - xr[1]], [xi[0] + xi[1], xi[0] - xi[1]]
    er, ei = _fft(xr[0::2], xi[0::2], sgn)
    ar, ai = _fft(xr[1::4], xi[1::4], sgn)
    br, bi = _fft(xr[3::4], xi[3::4], sgn)
    outr = [None] * n
    outi = [None] * n
    q = n // 4
    for k in range(q):
        a1 = sgn * 2 * math.pi * k / n
        a3 = 3 * a1
        z1r, z1i = _cmul(ar[k], ai[k], math.cos(a1), math.sin(a1))
        z3r, z3i = _cmul(br[k], bi[k], math.cos(a3), math.sin(a3))
        sr, si = z1r + z3r, z1i + z3i
        dr, di = z1r - z3r, z1i - z3i
        outr[k], outi[k] = er[k] + sr, ei[k] + si
        outr[k + 2 * q], outi[k + 2 * q] = er[k] - sr, ei[k] - si
        if sgn < 0:
            outr[k + q], outi[k + q] = er[k + q] + di, ei[k + q] - dr
            outr[k + 3 * q], outi[k + 3 * q] = er[k + q] - di, ei[k + q] + dr
        else:
            outr[k + q], outi[k + q] = er[k + q] - di, ei[k + q] + dr
            outr[k + 3 * q], outi[k + 3 * q] = er[k + q] + di, ei[k + q] - dr
    return outr, outi


def _rcp(l):
    if CFG['rcp_newton']:
        x = pl.reciprocal(l, approx=True)
        return x * (2.0 - l * x)
    return 1.0 / l


def _dot(a, b):
    return jnp.dot(a, b, preferred_element_type=f32)


def _kernel(xa_h, wrT_h, wiT_h, xb_h, wqkv_h, wo_h, mf_h, nf_h, g_h, h_h, out_h,
            xa_v, wrT_v, wiT_v, xb_v, wqkv_v, wo_v, mf_v, nf_v, g_v, h_v, oa_v, ob_v,
            mf_s, nf_s, u_s, st_s, wp_s,
            wqv_s, xb_s, wo_s, bias_s, z_s, wq_s, vw_s, kw_s, o_s,
            isem, osem, pad_s):
    def cp(src, dst, k):
        return pltpu.make_async_copy(src, dst, isem.at[k])

    def rows(ref, c, n):
        return ref.at[pl.ds(c * n, n), :]

    d_mf = cp(mf_h, mf_v, 0)
    d_xa = [cp(rows(xa_h, c, 1024), rows(xa_v, c, 1024), 1 + c) for c in range(2)]
    d_wk = cp(wqkv_h.at[:, D:2 * D], wqkv_v.at[:, D:2 * D], 5)
    d_xb = [cp(xb_h.at[lo:hi, :], xb_v.at[lo:hi, :], 18 + c) for c, (lo, hi) in
            enumerate(zip((0,) + CFG['xb_split'], CFG['xb_split'] + (S,)))]
    d_wq = cp(wqkv_h.at[:, 0:D], wqkv_v.at[:, 0:D], 10)
    d_wv = cp(wqkv_h.at[:, 2 * D:3 * D], wqkv_v.at[:, 2 * D:3 * D], 11)
    d_wr = [cp(wrT_h.at[:, c * 1024:(c + 1) * 1024], wrT_v.at[:, c * 1024:(c + 1) * 1024], 12 + 10 * c) for c in range(2)]
    d_wi = [cp(wiT_h.at[:, c * 1024:(c + 1) * 1024], wiT_v.at[:, c * 1024:(c + 1) * 1024], 13 + 10 * c) for c in range(2)]
    d_g = cp(g_h, g_v, 14)
    d_h = cp(h_h, h_v, 15)
    d_wo = cp(wo_h, wo_v, 16)
    d_nf = cp(nf_h, nf_v, 17)

    if CFG['w_early']:
        order = [d_mf, d_xa[0], d_xa[1], d_wr[0], d_wi[0], d_wq, d_wv, d_wr[1], d_wi[1]]
    else:
        order = [d_mf, d_xa[0], d_xa[1], d_wq, d_wv, d_wr[0], d_wi[0], d_wr[1], d_wi[1]]
    for d in [d_wk] + d_xb + order:
        d.start()
    late = (d_g, d_h, d_wo, d_nf)
    if CFG['b_late'] < 0:
        for d in late:
            d.start()

    def p1_block(i):
        r0 = pl.multiple_of(i * 128, 128)
        xt = [xa_v[pl.ds(r0, 128), t * 128:(t + 1) * 128].astype(f32) for t in range(5)]
        t1, t2 = xt[1] + xt[4], xt[2] + xt[3]
        t3, t4 = xt[1] - xt[4], xt[2] - xt[3]
        y0 = (xt[0] + t1 + t2).astype(bf16)
        y1r = (xt[0] + C1 * t1 + C2 * t2).astype(bf16)
        y2r = (xt[0] + C2 * t1 + C1 * t2).astype(bf16)
        y1i = ((-S1) * t3 - S2 * t4).astype(bf16)
        y2i = ((-S2) * t3 + S1 * t4).astype(bf16)
        for p, (yr, yi) in enumerate(((y1r, y1i), (y2r, y2i))):
            for n in range(2):
                m_r = unpk(mf_s[p * 128:p * 128 + 64, n * 128:(n + 1) * 128])
                m_i = unpk(mf_s[p * 128 + 64:p * 128 + 128, n * 128:(n + 1) * 128])
                u_s[p + 3 * n, pl.ds(r0, 128), :] = _dot(yr, m_r) + _dot(yi, m_i)
        e = _dot(y0, unpk(mf_s[256:320, 0:128]))
        lane = jax.lax.broadcasted_iota(i32, (128, 128), 1)
        u_s[2, pl.ds(r0, 128), :] = e
        u_s[5, pl.ds(r0, 128), :] = jnp.where((lane & 63) == 0, 0.0, pltpu.roll(e, 64, 1))

    def fft_set(p, r, sgn, toks=None):
        off = pl.multiple_of(r * 8, 8)
        xr = [u_s[p, pl.ds(64 * n + off, 8), :] for n in range(32)]
        xi = [u_s[3 + p, pl.ds(64 * n + off, 8), :] for n in range(32)]
        if toks is not None:
            for n in range(16):
                tk = toks[0] if n % 2 == 0 else (toks[1] if n % 4 == 1 else toks[2])
                xr[n] = pltpu.bitcast(pltpu.bitcast(xr[n], i32) | tk, f32)
                xi[n] = pltpu.bitcast(pltpu.bitcast(xi[n], i32) | tk, f32)
        yr, yi = _fft(xr, xi, sgn)
        for n in range(32):
            u_s[p, pl.ds(64 * n + off, 8), :] = yr[n]
            u_s[3 + p, pl.ds(64 * n + off, 8), :] = yi[n]

    def wprep(T, tk):
        c0 = pl.multiple_of(T * 128, 128)
        q0 = pl.multiple_of(T * 64, 64)
        zer = jnp.zeros((56, 128), f32)
        sub = jax.lax.broadcasted_iota(i32, (8, 128), 0)
        for j, ref in enumerate((wrT_v, wiT_v)):
            wv = pk(ref[0:320, pl.ds(c0, 128)])
            wv = (wv.reshape(20, 8, 128) | pltpu.bitcast(tk[j], u32)[None]).reshape(160, 128)
            jj = j + (2 * (T % 2) if CFG['st_dbl'] and isinstance(T, int) else 0)
            st_s[jj, 0:320, :] = unpk(wv).astype(f32)
            last = jnp.broadcast_to(ref[320:321, pl.ds(c0, 128)].astype(f32), (8, 128))
            last = jnp.where(sub == 0, last, 0.0)
            sl = lambda a: st_s[jj, pl.ds(a, 64, stride=5), :]
            tiles = (jnp.concatenate([sl(1), sl(4)], axis=0),
                     jnp.concatenate([sl(2), sl(3)], axis=0),
                     jnp.concatenate([sl(0), last, zer], axis=0))
            for p in range(3):
                wp_s[3 * j + p, pl.ds(q0, 64), :] = pk(tiles[p].astype(bf16).T)

    def mid_pair(a):
        wv = [wp_s[t, pl.ds(a, 64, stride=16), :] for t in range(6)]
        for j in range(2):
            k1 = 2 * a + j
            r0 = pl.multiple_of(k1 * 64, 64)
            if j == 0:
                wf = [pltpu.bitcast(w << 16, f32) for w in wv]
            else:
                wf = [pltpu.bitcast(w & jnp.uint32(0xFFFF0000), f32) for w in wv]
            gk, hk = g_v[k1], h_v[k1]
            for p in range(3):
                y = jnp.concatenate([u_s[p, pl.ds(r0, 64), :], u_s[3 + p, pl.ds(r0, 64), :]], axis=0).astype(bf16)
                x = _dot(gk, y)
                xr, xi = x[0:64], x[64:128]
                wr, wi = wf[p], wf[3 + p]
                pp = jnp.concatenate([xr * wr - xi * wi, xr * wi + xi * wr], axis=0).astype(bf16)
                z = _dot(hk, pp)
                u_s[p, pl.ds(r0, 64), :] = z[0:64]
                u_s[3 + p, pl.ds(r0, 64), :] = z[64:128]

    def p5_block(i, tk=None):
        r0 = pl.multiple_of(i * 128, 128)
        z = [u_s[t, pl.ds(r0, 128), :] for t in range(6)]
        if tk is not None:
            z = [jnp.concatenate([pltpu.bitcast(pltpu.bitcast(a[0:8], i32) | tk, f32), a[8:128]], axis=0) for a in z]
        lane = jax.lax.broadcasted_iota(i32, (128, 128), 1)
        ze = jnp.where(lane <= 64, z[2], pltpu.roll(z[5], 64, 1)).astype(bf16)
        z = [a.astype(bf16) for a in z]

        def prod(p, c0):
            return (_dot(z[p], unpk(nf_s[0:64, c0:c0 + 128])) + _dot(z[3 + p], unpk(nf_s[64:128, c0:c0 + 128])))
        r1, i1 = prod(0, 0), prod(0, 128)
        r2, i2 = prod(1, 256), prod(1, 384)
        t0 = _dot(ze, unpk(nf_s[0:64, 512:640]))
        a1 = t0 + C1 * r1 + C2 * r2
        b1 = S1 * i1 + S2 * i2
        a2 = t0 + C2 * r1 + C1 * r2
        b2 = S2 * i1 - S1 * i2
        ys = (t0 + r1 + r2, a1 - b1, a2 - b2, a2 + b2, a1 + b1)
        for t in range(5):
            oa_v[pl.ds(r0, 128), t * 128:(t + 1) * 128] = ys[t].astype(bf16)
        pltpu.make_async_copy(oa_v.at[pl.ds(r0, 128), :], out_h.at[pl.ds(r0, 128), 0:D], osem.at[0, i]).start()

    def setup_misc():
        row = jax.lax.broadcasted_iota(i32, (128, 128), 0)
        lane = jax.lax.broadcasted_iota(i32, (128, 128), 1)
        bias_s[0] = jnp.where(row > lane, 0.0, NEG).astype(f32)
        bias_s[1] = jnp.zeros((128, 128), f32)
        bias_s[2] = jnp.where(row <= lane, 0.0, NEG).astype(f32)
        okm = jnp.where(row < 64, jnp.where(lane < 64, lane - row, row - lane + 63),
                        jnp.where(lane < 64, -1, lane - row))
        bias_s[3] = jnp.where(okm < 0, 0.0, NEG).astype(f32)
        bias_s[4] = jnp.where(jnp.where(row < 64, row - lane - 1, lane - row) < 0, 0.0, NEG).astype(f32)
        r5, q5 = row & 31, lane & 31
        grp, lg = row >> 5, lane >> 5
        bad5 = (((grp == 0) & (lg == 0) & (r5 > q5)) | ((grp == 1) & (lg == 3) & (r5 <= q5))
                | ((grp == 2) & (lg == 1) & (r5 > q5)) | ((grp == 3) & (lg == 2) & (r5 <= q5)))
        bias_s[5] = jnp.where(bad5, NEG, 0.0).astype(f32)
        bad6 = jnp.where(lg < 2, q5 - r5, r5 - q5 - 1) >= 0
        bias_s[6] = jnp.where(bad6, NEG, 0.0).astype(f32)
        z_s[...] = jnp.zeros(z_s.shape, i32)

    def proj_k(i):
        r0 = pl.multiple_of(i * 128, 128)
        xi = xb_v[pl.ds(r0, 128), :]
        xb_s[i] = pk(xi)
        tiles = []
        for n in range(5):
            acc = None
            for kt in range(5):
                r = _dot(xi[:, kt * 128:(kt + 1) * 128], wqkv_v[kt * 128:(kt + 1) * 128, D + n * 128:D + (n + 1) * 128])
                acc = r if acc is None else acc + r
            tiles.append(pk(acc.astype(bf16)))
        lane = jax.lax.broadcasted_iota(i32, (64, 128), 1)
        for g in range(8):
            off = (80 * g) % 128
            ta = (80 * g) // 128
            if off == 0:
                w = tiles[ta]
            else:
                w = pltpu.roll(tiles[ta], 128 - off, 1)
                if off + 80 > 128:
                    w = jnp.where(lane < 128 - off, w, pltpu.roll(tiles[ta + 1], 128 - off, 1))
            kw_s[i, :, g * 128:(g + 1) * 128] = w

    def proj_qv(i):
        xi = unpk(xb_s[i])
        toks = []
        zero = z_s[...]

        def part(c0):
            outs = []
            for n in range(5):
                acc = None
                for kt in range(5):
                    r = _dot(xi[:, kt * 128:(kt + 1) * 128],
                             unpk(wqv_s[kt * 64:(kt + 1) * 64, c0 + n * 128:c0 + (n + 1) * 128]))
                    if kt == 0:
                        toks.append(pltpu.bitcast(r[0:8], i32) & zero)
                    acc = r if acc is None else acc + r
                outs.append(acc)
            return outs
        sub = jax.lax.broadcasted_iota(i32, (16, 128), 0)
        qT = jnp.concatenate([pk((a * SCALE).astype(bf16).T) for a in part(0)], axis=0)
        for h in range(H):
            r0 = (20 * h) // 16 * 8
            dl = (20 * h) % 16 // 2
            wq_s[i, h] = jnp.where((sub >= dl) & (sub < dl + 10), qT[r0:r0 + 16], jnp.uint32(0))
        vT = jnp.concatenate([pk(a.astype(bf16).T) for a in part(D)], axis=0)
        one = jnp.uint32(0x3F803F80)
        for h in range(H):
            r0 = (20 * h) // 16 * 8
            dl = (20 * h) % 16 // 2
            if dl <= 2:
                w = jnp.concatenate([vT[r0:r0 + 8], jnp.where(sub[0:8] >= 4, one, vT[r0 + 8:r0 + 16])], axis=0)
            else:
                w = jnp.concatenate([jnp.where(sub[0:8] < 4, one, vT[r0:r0 + 8]), vT[r0 + 8:r0 + 16]], axis=0)
            vw_s[i, h] = w
        return toks

    def out_proj(i, tokz=None, tiles=(0, 1, 2, 3, 4)):
        r0 = pl.multiple_of(i * 128, 128)
        ot = [o_s[i, :, n * 128:(n + 1) * 128] for n in range(5)]
        if tokz is not None:
            ot = [(o.reshape(8, 8, 128) | pltpu.bitcast(tokz, u32)[None]).reshape(64, 128) for o in ot]
        ot = [unpk(o) for o in ot]
        for n in tiles:
            acc = None
            for kt in range(5):
                r = _dot(ot[kt], unpk(wo_s[kt * 64:(kt + 1) * 64, n * 128:(n + 1) * 128]))
                acc = r if acc is None else acc + r
            ob_v[pl.ds(r0, 128), n * 128:(n + 1) * 128] = acc.astype(bf16)
        if 4 in tiles:
            pltpu.make_async_copy(ob_v.at[pl.ds(r0, 128), :], out_h.at[pl.ds(r0, 128), D:2 * D], osem.at[1, i]).start()

    def attention(jobs, lag=5, drain=None):
        zero = z_s[...]
        seq = []
        info = []
        for jb, rounds in enumerate(jobs):
            nr = len(rounds)
            slots = sorted(set(r[3] for r in rounds))
            last = {s: max(t for t in range(nr) if rounds[t][3] == s) for s in slots}
            first = {s: min(t for t in range(nr) if rounds[t][3] == s) for s in slots}
            info.append((rounds, slots, first, last))
            for g in range(8):
                for t in range(nr):
                    seq.append((jb, g, t))

        def getw(qb, g, h):
            o = 20 * h - 80 * g
            r0 = o // 16 * 16
            parts = []
            if r0 > 0:
                parts.append(jnp.zeros((r0, 128), bf16))
            parts.append(unpk(wq_s[qb, h]))
            if 96 - r0 > 0:
                parts.append(jnp.zeros((96 - r0, 128), bf16))
            return jnp.concatenate(parts, axis=0)
        sv, mx, acc, tok, res = {}, {}, {}, {}, {}

        def qk(k):
            jb, g, t = seq[k]
            rounds, slots, first, last = info[jb]
            qb, kb, bi, sl = rounds[t]
            kk = unpk(kw_s[kb, :, g * 128:(g + 1) * 128])
            for j, h in enumerate(range(4 * g, 4 * g + 4)):
                key = (jb, sl, h)
                st = _dot(kk, getw(qb, g, h))
                tok[(k, j)] = pltpu.bitcast(st[0:8], i32) & zero
                if bi is not None:
                    st = st + bias_s[bi]
                sv[(k, j)] = st
                mm = jnp.max(st.reshape(16, 8, 128), axis=0)
                mx[key] = mm if t == first[sl] else jnp.maximum(mx[key], mm)
                if t == last[sl]:
                    mx[key] = jnp.broadcast_to(jnp.max(mx[key], axis=0, keepdims=True), (8, 128))

        def finish(jb):
            rounds, slots, first, last = info[jb]
            sub = jax.lax.broadcasted_iota(i32, (8, 128), 0)
            for sl in slots:
                qb = rounds[first[sl]][0]
                vregs = []
                for v in range(80):
                    h0, h1 = (8 * v) // 20, (8 * v + 7) // 20

                    def get(h):
                        r0 = (20 * h) // 16 * 16
                        return res[(jb, sl, h)][8 * v - r0:8 * v - r0 + 8]
                    vregs.append(get(h0) if h0 == h1 else jnp.where(sub < (20 * h1 - 8 * v), get(h0), get(h1)))
                oT = jnp.concatenate(vregs, axis=0).astype(bf16)
                for n in range(5):
                    o_s[qb, :, n * 128:(n + 1) * 128] = pk(oT[n * 128:(n + 1) * 128].T)

        def pv(k, kt):
            jb, g, t = seq[k]
            rounds, slots, first, last = info[jb]
            qb, kb, bi, sl = rounds[t]
            ptok = None
            for j, h in enumerate(range(4 * g, 4 * g + 4)):
                key = (jb, sl, h)
                m = mx[key]
                if kt is not None:
                    m = pltpu.bitcast(pltpu.bitcast(m, i32) | tok[(kt, j)], f32)
                s = sv.pop((k, j))
                p = jnp.exp2(s.reshape(16, 8, 128) - m[None]).reshape(128, 128).astype(bf16)
                r = _dot(unpk(vw_s[kb, h]), p)
                if j == 3:
                    ptok = pltpu.bitcast(pk(p)[56:64], i32) & zero
                acc[key] = r if t == first[sl] else acc[key] + r
                if t == last[sl]:
                    dl = 20 * h % 16
                    a = acc.pop(key)
                    l = a[24:32] if dl <= 4 else a[0:8]
                    res[key] = (a.reshape(4, 8, 128) * _rcp(l)[None]).reshape(32, 128)
            if g == 7 and t == len(rounds) - 1:
                finish(jb)
            return ptok
        nk = len(seq)
        for k in range(nk + lag):
            if k < nk:
                qk(k)
            if k - lag >= 0:
                kt = k - 1
                if kt >= nk or kt < 0:
                    kt = None
                pt = pv(k - lag, kt)
                if drain is not None and k - nk + 1 in drain and k >= nk:
                    drain[k - nk + 1](pt)
            if k == nk - 1 and drain is not None and 0 in drain:
                drain[0](tok[(nk - 1, 3)])

    def attention2(blocks, lag=5, drain=None, pre=None):
        zero = z_s[...]
        lane = jax.lax.broadcasted_iota(i32, (32, 128), 1)
        lane16 = jax.lax.broadcasted_iota(i32, (16, 128), 1)
        lane8 = jax.lax.broadcasted_iota(i32, (8, 128), 1)
        seq = [(jb, g, t) for jb in range(len(blocks)) for g in range(8) for t in range(3)]
        zq = jnp.zeros((16, 128), bf16)

        def place(parts):
            out, pos = [], 0
            for r0, w in parts:
                out += [zq] * ((r0 - pos) // 16) + [w]
                pos = r0 + 32
            out += [zq] * ((128 - pos) // 16)
            return jnp.concatenate(out, axis=0)
        sv, mx, acc, tok, res = {}, {}, {}, {}, {}

        def qk(k):
            jb, g, t = seq[k]
            i = blocks[jb]
            cs = slice(g * 128, (g + 1) * 128)
            if t == 0:
                kk = unpk(kw_s[i - 1, :, cs])
            elif t == 1:
                kk = unpk(jnp.concatenate([kw_s[i, 0:32, cs], kw_s[i - 2, 32:64, cs]], axis=0))
            else:
                ka = kw_s[i - 2, 0:32, cs]
                kr = pltpu.roll(kw_s[i, 32:64, cs], 48, 1)
                km = [unpk(jnp.where(lane < 44, ka, kr)), unpk(jnp.where(lane < 84, ka, kr))]
            for j, h in enumerate(range(4 * g, 4 * g + 4)):
                key = (jb, h)
                r0 = 20 * j // 16 * 16
                w32 = wq_s[i, h]
                if t == 2:
                    wm = place([(r0, unpk(jnp.where(lane16 < 64, w32, jnp.uint32(0)))),
                                (r0 + 48, unpk(jnp.where(lane16 >= 64, w32, jnp.uint32(0))))])
                    st = _dot(km[j // 2], wm)
                else:
                    st = _dot(kk, place([(r0, unpk(w32))]))
                tok[(k, j)] = pltpu.bitcast(st[0:8], i32) & zero
                if t == 1:
                    st = st + bias_s[4]
                elif t == 2:
                    st = st + bias_s[3, 0:64]
                sv[(k, j)] = st
                mm = jnp.max(st.reshape(-1, 8, 128), axis=0)
                mx[key] = mm if t == 0 else jnp.maximum(mx[key], mm)
                if t == 2:
                    mx[key] = jnp.broadcast_to(jnp.max(mx[key], axis=0, keepdims=True), (8, 128))

        def finish(jb):
            sub = jax.lax.broadcasted_iota(i32, (8, 128), 0)
            vregs = []
            for v in range(80):
                h0, h1 = (8 * v) // 20, (8 * v + 7) // 20

                def get(h):
                    r0 = (20 * h) // 16 * 16
                    return res[(jb, h)][8 * v - r0:8 * v - r0 + 8]
                vregs.append(get(h0) if h0 == h1 else jnp.where(sub < (20 * h1 - 8 * v), get(h0), get(h1)))
            oT = jnp.concatenate(vregs, axis=0).astype(bf16)
            for n in range(5):
                o_s[blocks[jb], :, n * 128:(n + 1) * 128] = pk(oT[n * 128:(n + 1) * 128].T)

        def pv(k, kt):
            jb, g, t = seq[k]
            i = blocks[jb]
            ptok = None
            for j, h in enumerate(range(4 * g, 4 * g + 4)):
                key = (jb, h)
                m = mx[key]
                if kt is not None:
                    m = pltpu.bitcast(pltpu.bitcast(m, i32) | tok[(kt, j)], f32)
                s = sv.pop((k, j))
                pf = jnp.exp2(s.reshape(-1, 8, 128) - m[None]).reshape(-1, 128)
                p = pf.astype(bf16)
                if t == 0:
                    acc[key] = _dot(unpk(vw_s[i - 1, h]), p)
                elif t == 1:
                    v = jnp.where(lane16 < 64, vw_s[i, h], vw_s[i - 2, h])
                    acc[key] = acc[key] + _dot(unpk(v), p)
                else:
                    v = jnp.where(lane16 < 64, vw_s[i - 2, h], vw_s[i, h])
                    l64 = jax.lax.broadcasted_iota(i32, (64, 128), 1)
                    pw = jnp.concatenate([jnp.where(l64 < 64, pf, 0.0), jnp.where(l64 >= 64, pf, 0.0)], axis=0)
                    a = acc.pop(key) + _dot(unpk(v), pw.astype(bf16))
                    dl = 20 * h % 16
                    l = a[24:32] if dl <= 4 else a[0:8]
                    res[key] = (a.reshape(4, 8, 128) * _rcp(l)[None]).reshape(32, 128)
                if j == 3:
                    ptok = pltpu.bitcast(pf[56:64], i32) & zero
            if g == 7 and t == 2:
                finish(jb)
            return ptok
        nk = len(seq)
        assert drain is None or max(drain) <= lag
        for k in range(nk + lag):
            if k < nk:
                qk(k)
            if k - lag >= 0:
                kt = k - CFG['tokoff']
                if kt >= nk or kt < 0:
                    kt = None
                pt = pv(k - lag, kt)
                if drain is not None and k - nk + 1 in drain and k != nk - 1:
                    drain[k - nk + 1](pt)
            if k == nk - CFG['dtok'] and drain is not None and 0 in drain:
                drain[0](tok[(k, 3)])
            if pre is not None and k in pre:
                pre[k](tok[(k, 0)])

    def attention3(blocks, lag=5, drain=None, pre=None):
        zero = z_s[...]
        zu = jnp.uint32(0)

        def lanes(n):
            return jax.lax.broadcasted_iota(i32, (n, 128), 1)
        seq = [(jb, g, t) for jb in range(len(blocks)) for g in range(8) for t in range(3)]
        zq = jnp.zeros((16, 128), bf16)

        def place(parts):
            out, pos = [], 0
            for r0, w in parts:
                out += [zq] * ((r0 - pos) // 16) + [unpk(w)]
                pos = r0 + 32
            out += [zq] * ((128 - pos) // 16)
            return jnp.concatenate(out, axis=0)

        def roll(x, a):
            return x if a % 128 == 0 else pltpu.roll(x, a % 128, 1)
        sv, pp, mx, acc, tok, res = {}, {}, {}, {}, {}, {}

        def qk(k):
            jb, g, t = seq[k]
            i = blocks[jb]
            cs = slice(g * 128, (g + 1) * 128)
            l16 = lanes(16)
            if t == 0:
                kk = unpk(kw_s[i - 1, :, cs])
            elif t == 1:
                kk = unpk(jnp.concatenate([kw_s[i, 0:16, cs], kw_s[i - 2, 48:64, cs]], axis=0))
                ka = kw_s[i - 2, 16:48, cs]
                kr = pltpu.roll(kw_s[i, 16:48, cs], 48, 1)
                km = [unpk(jnp.where(lanes(32) < 44, ka, kr)), unpk(jnp.where(lanes(32) < 84, ka, kr))]
            else:
                kc = [kw_s[i - 2, 0:16, cs], kw_s[i - 2, 16:32, cs], kw_s[i, 32:48, cs], kw_s[i, 48:64, cs]]
                if CFG['kc_gate']:
                    tz = pltpu.bitcast(tok[(k - CFG['kc_gate'], 0)], u32) if k >= CFG['kc_gate'] else None
                    if tz is not None:
                        kc = [(x.reshape(2, 8, 128) | tz[None]).reshape(16, 128) for x in kc]
            for j, h in enumerate(range(4 * g, 4 * g + 4)):
                key = (jb, h)
                r0 = 20 * j // 16 * 16
                w32 = wq_s[i, h]
                if t == 0:
                    st = _dot(kk, place([(r0, w32)]))
                    tok[(k, j)] = pltpu.bitcast(st[0:8], i32) & zero
                elif t == 1:
                    def wsplit(thr):
                        return place([(r0, jnp.where(l16 < thr, w32, zu)), (r0 + 48, jnp.where(l16 >= thr, w32, zu))])
                    sp = _dot(kk, place([(r0, w32)]))
                    tok[(k, j)] = pltpu.bitcast(sp[0:8], i32) & zero
                    st = [sp + bias_s[5, 0:64], _dot(km[j // 2][0:32], wsplit(32)) + bias_s[5, 64:96],
                          _dot(km[j // 2][32:64], wsplit(96)) + bias_s[5, 96:128]]
                else:
                    c = roll(kc[3], 96 - r0)
                    for s in (2, 1, 0):
                        c = jnp.where(l16 < 32 * s + 32, roll(kc[s], 32 * s - r0), c)
                    w4 = place([(32 * s, jnp.where((l16 >> 5) == s, w32, zu)) for s in range(4)])
                    st = _dot(unpk(c), w4)
                    tok[(k, j)] = pltpu.bitcast(st[0:8], i32) & zero
                    st = st + bias_s[6, 0:32]
                if not isinstance(st, list):
                    st = [st]
                sv[(k, j)] = st
                mm = functools.reduce(jnp.maximum, [jnp.max(x.reshape(-1, 8, 128), axis=0) for x in st])
                mx[key] = mm if t == 0 else jnp.maximum(mx[key], mm)
                if t == 2:
                    mx[key] = jnp.broadcast_to(jnp.max(mx[key], axis=0, keepdims=True), (8, 128))

        def finish(jb):
            sub = jax.lax.broadcasted_iota(i32, (8, 128), 0)
            vregs = []
            for v in range(80):
                h0, h1 = (8 * v) // 20, (8 * v + 7) // 20

                def get(h):
                    r0 = (20 * h) // 16 * 16
                    return res[(jb, h)][8 * v - r0:8 * v - r0 + 8]
                vregs.append(get(h0) if h0 == h1 else jnp.where(sub < (20 * h1 - 8 * v), get(h0), get(h1)))
            oT = jnp.concatenate(vregs, axis=0).astype(bf16)
            for n in range(5):
                o_s[blocks[jb], :, n * 128:(n + 1) * 128] = pk(oT[n * 128:(n + 1) * 128].T)

        def pv(k, kt):
            jb, g, t = seq[k]
            i = blocks[jb]
            ptok = None
            l16 = lanes(16)
            for j, h in enumerate(range(4 * g, 4 * g + 4)):
                key = (jb, h)
                m = mx[key]
                if kt is not None:
                    m = pltpu.bitcast(pltpu.bitcast(m, i32) | tok[(kt, j)], f32)
                s = sv.pop((k, j))
                if t == 1:
                    s = [s[0][0:32], s[0][32:64], s[1], s[2]]
                ps = [jnp.exp2(x.reshape(-1, 8, 128) - m[None]).reshape(-1, 128) for x in s]
                if t == 0:
                    acc[key] = _dot(unpk(vw_s[i - 1, h]), ps[0].astype(bf16))
                elif t == 1:
                    pp[key] = ps
                else:
                    pc = ps[0]
                    d0, f3, m1, m2 = pp.pop(key)
                    l32 = lanes(32)
                    far = jnp.concatenate([jnp.where(l32 < 32, pc, 0.0),
                                           jnp.where(l32 < 32, m1, jnp.where(l32 < 64, pc, 0.0)),
                                           jnp.where(l32 < 96, m2, 0.0), f3], axis=0).astype(bf16)
                    dia = jnp.concatenate([d0, jnp.where(l32 >= 32, m1, 0.0),
                                           jnp.where(l32 >= 96, m2, jnp.where(l32 >= 64, pc, 0.0)),
                                           jnp.where(l32 >= 96, pc, 0.0)], axis=0).astype(bf16)
                    a = acc.pop(key) + _dot(unpk(vw_s[i - 2, h]), far) + _dot(unpk(vw_s[i, h]), dia)
                    dl = 20 * h % 16
                    l = a[24:32] if dl <= 4 else a[0:8]
                    res[key] = (a.reshape(4, 8, 128) * _rcp(l)[None]).reshape(32, 128)
                if j == 3:
                    ptok = pltpu.bitcast(ps[-1][24:32], i32) & zero
            if g == 7 and t == 2:
                finish(jb)
            return ptok
        nk = len(seq)
        assert drain is None or max(drain) <= lag
        for k in range(nk + lag):
            if k < nk:
                qk(k)
            if k - lag >= 0:
                kt = k - CFG['tokoff']
                if kt >= nk or kt < 0:
                    kt = None
                pt = pv(k - lag, kt)
                if drain is not None and k - nk + 1 in drain and k != nk - 1:
                    drain[k - nk + 1](pt)
            if k == nk - CFG['dtok'] and drain is not None and 0 in drain:
                drain[0](tok[(k, 3)])
            if pre is not None and k in pre:
                pre[k](tok[(k, 0)])

    setup_misc()

    if True:
        d_wk.wait()
        bounds = {lo // 128: c for c, lo in enumerate((0,) + CFG['xb_split'])}
        if CFG['k_loop'] == 1:
            for j in range(NB):
                if j in bounds:
                    d_xb[bounds[j]].wait()
                proj_k(j)
        else:
            per = NB // CFG['k_loop']

            def loop_k(it, carry):
                for j in range(per):
                    for t in range(CFG['k_loop']):
                        if t * per + j in bounds:
                            pl.when(it == t)(lambda c=bounds[t * per + j]: d_xb[c].wait())
                    proj_k(per * it + j)
                return carry
            jax.lax.fori_loop(0, CFG['k_loop'], loop_k, 0)

    if True:
        d_mf.wait()
        d_xa[0].wait()
        d_xa[1].wait()
        if CFG['w_early']:
            d_wr[0].wait()
            d_wi[0].wait()
        mf_s[...] = pk(mf_v[...])
        for j in range(NB):
            if j == CFG['a_conv']:
                d_wq.wait()
                d_wv.wait()
                wqv_s[:, 0:D] = pk(wqkv_v[:, 0:D])
                wqv_s[:, D:2 * D] = pk(wqkv_v[:, 2 * D:3 * D])
            p1_block(j)
        if CFG['a_conv'] >= NB:
            d_wq.wait()
            d_wv.wait()
            wqv_s[:, 0:D] = pk(wqkv_v[:, 0:D])
            wqv_s[:, D:2 * D] = pk(wqkv_v[:, 2 * D:3 * D])

    def phase_b(q):
        tk = proj_qv(q)
        for j in range(3):
            fft_set(j, q, -1, tk[3 * j:3 * j + 3])
        wprep(2 * q, tk[1:3])
        wprep(2 * q + 1, tk[6:8])

    def phase_d(q):
        tk = proj_qv(8 + q)
        for j in range(3):
            fft_set(j, q, +1, tk[3 * j:3 * j + 3])

    def rep(fn, n, iters):
        if iters == 1:
            for q in range(n):
                fn(q)
        else:
            per = n // iters

            def body(it, carry):
                for q in range(per):
                    fn(per * it + q)
                return carry
            jax.lax.fori_loop(0, iters, body, 0)

    if True:
        if not CFG['w_early']:
            d_wr[0].wait()
            d_wi[0].wait()
        for q in range(8):
            if q == CFG['b_late']:
                for d in late:
                    d.start()
            if q == 4:
                d_wr[1].wait()
                d_wi[1].wait()
                if CFG['late_mid']:
                    for d in late:
                        d.wait()
                    wo_s[...] = pk(wo_v[...])
                    nf_s[...] = pk(nf_v[...])
            phase_b(q)
        if not CFG['late_mid']:
            for d in late:
                d.wait()
            wo_s[...] = pk(wo_v[...])
            nf_s[...] = pk(nf_v[...])

    if True:
        rep(mid_pair, 16, CFG['c_mode'])

    if True:
        rep(phase_d, 8, 1 if CFG['d_mode'] == "line" else CFG['d_mode'])

    if True:
        p5_block(0)
        attention([[(0, 0, 2, 0), (1, 0, None, 1), (1, 1, 2, 1)]], drain={0: lambda tz: p5_block(1, tz)})

    def loop_e(it, carry):
        if CFG['e_un'] == 2:
            i = 2 * it
            pre = None
            if CFG['p5_pre'] is None:
                p5_block(i)
            else:
                pre = {CFG['p5_pre']: lambda tz: p5_block(i, tz)}
            if CFG['p5b_pre'] is not None:
                pre[CFG['p5b_pre']] = lambda tz: p5_block(i + 1, tz)
            p5b = (lambda tz: None) if CFG['p5b_pre'] is not None else (lambda tz: p5_block(i + 1, tz))
            if CFG['drain'] == "full":
                drain = {0: lambda tz: (out_proj(i - 2, tz), out_proj(i - 1, tz), p5_block(i + 1, tz))}
            elif CFG['drain'] == "ladder":
                drain = {0: lambda tz: out_proj(i - 2, tz, (0, 1)),
                         1: lambda tz: out_proj(i - 2, tz, (2, 3)),
                         2: lambda tz: out_proj(i - 2, tz, (4,)),
                         3: lambda tz: out_proj(i - 1, tz, (0, 1)),
                         4: lambda tz: (p5b(tz), out_proj(i - 1, tz, (2, 3, 4)))}
            elif CFG['drain'] == "ladder2":
                drain = {0: lambda tz: out_proj(i - 2, tz),
                         2: lambda tz: out_proj(i - 1, tz),
                         4: lambda tz: p5_block(i + 1, tz)}
            elif CFG['drain'] == "ladder3":
                drain = {0: lambda tz: out_proj(i - 2, tz, (0, 1, 2)),
                         1: lambda tz: out_proj(i - 2, tz, (3, 4)),
                         2: lambda tz: out_proj(i - 1, tz, (0, 1)),
                         3: lambda tz: out_proj(i - 1, tz, (2,)),
                         4: lambda tz: (p5_block(i + 1, tz), out_proj(i - 1, tz, (3, 4)))}
            elif CFG['drain'] == "ladder4":
                drain = {0: lambda tz: out_proj(i - 2, tz, (0, 1)),
                         1: lambda tz: out_proj(i - 2, tz, (2, 3)),
                         2: lambda tz: (out_proj(i - 2, tz, (4,)), p5_block(i + 1, tz)),
                         3: lambda tz: out_proj(i - 1, tz, (0, 1)),
                         4: lambda tz: out_proj(i - 1, tz, (2, 3, 4))}
            elif CFG['drain'] == "ladder5":
                drain = {0: lambda tz: out_proj(i - 2, tz, (0, 1)),
                         1: lambda tz: out_proj(i - 2, tz, (2, 3)),
                         2: lambda tz: out_proj(i - 2, tz, (4,)),
                         3: lambda tz: out_proj(i - 1, tz, (0, 1)),
                         4: lambda tz: out_proj(i - 1, tz, (2,)),
                         5: lambda tz: (p5b(tz), out_proj(i - 1, tz, (3, 4)))}
            elif CFG['drain'] == "ladder6":
                drain = {0: lambda tz: out_proj(i - 2, tz, (0, 1)),
                         2: lambda tz: out_proj(i - 2, tz, (2, 3)),
                         3: lambda tz: out_proj(i - 2, tz, (4,)),
                         4: lambda tz: out_proj(i - 1, tz, (0, 1)),
                         5: lambda tz: (p5b(tz), out_proj(i - 1, tz, (2, 3, 4)))}
            elif CFG['drain'] == "keys":
                ks = CFG['dkeys']
                parts = [lambda tz: out_proj(i - 2, tz, (0, 1)), lambda tz: out_proj(i - 2, tz, (2, 3)),
                         lambda tz: out_proj(i - 2, tz, (4,)), lambda tz: out_proj(i - 1, tz, (0, 1)),
                         lambda tz: out_proj(i - 1, tz, (2,)), lambda tz: out_proj(i - 1, tz, (3, 4)), p5b]
                drain = {}
                for kk_ in sorted(set(ks)):
                    fs = [f for f, q_ in zip(parts, ks) if q_ == kk_]
                    drain[kk_] = (lambda tz, fs=fs: [f(tz) for f in fs])
            elif CFG['drain'] == "ladder7":
                drain = {0: lambda tz: out_proj(i - 2, tz, (0, 1, 2)),
                         2: lambda tz: out_proj(i - 2, tz, (3,)),
                         3: lambda tz: out_proj(i - 2, tz, (4,)),
                         4: lambda tz: out_proj(i - 1, tz, (0, 1)),
                         5: lambda tz: (p5b(tz), out_proj(i - 1, tz, (2, 3, 4)))}
            elif CFG['drain'] == "ladder8":
                drain = {0: lambda tz: out_proj(i - 2, tz, (0, 1)),
                         2: lambda tz: out_proj(i - 2, tz, (2, 3)),
                         3: lambda tz: out_proj(i - 2, tz, (4,)),
                         4: lambda tz: out_proj(i - 1, tz, (0, 1, 2)),
                         5: lambda tz: (p5b(tz), out_proj(i - 1, tz, (3, 4)))}
            elif CFG['drain'] == "ladder9":
                drain = {0: lambda tz: out_proj(i - 2, tz, (0,)),
                         1: lambda tz: out_proj(i - 2, tz, (1,)),
                         2: lambda tz: out_proj(i - 2, tz, (2, 3)),
                         3: lambda tz: out_proj(i - 2, tz, (4,)),
                         4: lambda tz: out_proj(i - 1, tz, (0, 1)),
                         5: lambda tz: (p5b(tz), out_proj(i - 1, tz, (2, 3, 4)))}
            elif CFG['drain'] == "mid":
                drain = {0: lambda tz: out_proj(i - 2, tz, (0, 1, 2)),
                         1: lambda tz: out_proj(i - 2, tz, (3, 4)),
                         2: lambda tz: out_proj(i - 1, tz, (0, 1)),
                         4: lambda tz: out_proj(i - 1, tz, (2, 3, 4)),
                         -20: lambda tz: p5_block(i + 1, tz)}
            (attention3 if CFG['g4'] else attention2)([i, i + 1], lag=CFG['lag'], drain=drain, pre=pre)
        else:
            i = it
            p5_block(i)
            drain = {0: lambda tz: out_proj(i - 2, tz, (0, 1)),
                     1: lambda tz: out_proj(i - 2, tz, (2,)),
                     2: lambda tz: out_proj(i - 2, tz, (3,)),
                     CFG['lag']: lambda tz: out_proj(i - 2, tz, (4,))}
            attention2([i], lag=CFG['lag'], drain=drain)
        return carry
    if True:
        if CFG['e_un'] == 2:
            jax.lax.fori_loop(1, NB // 2, loop_e, 0)
        else:
            jax.lax.fori_loop(2, NB, loop_e, 0)
    if True:
        out_proj(NB - 2)
        out_proj(NB - 1)

    def loop_f(i, carry):
        r0 = pl.multiple_of(i * 128, 128)
        pltpu.make_async_copy(oa_v.at[pl.ds(r0, 128), :], out_h.at[pl.ds(r0, 128), 0:D], osem.at[0, i]).wait()
        pltpu.make_async_copy(ob_v.at[pl.ds(r0, 128), :], out_h.at[pl.ds(r0, 128), D:2 * D], osem.at[1, i]).wait()
        return carry
    if True:
        jax.lax.fori_loop(0, NB, loop_f, 0)


_CONSTS = _make_consts()


@jax.jit
def pallas_concat_heads__spectral_gfnet__sliding_block__prompt_kernel(A_x, A_w_r, A_w_i, B_x, B_wqkv, B_wo):
    mf, nf, g, hm = _CONSTS
    vm = pltpu.VMEM
    out = pl.pallas_call(
        _kernel,
        out_shape=jax.ShapeDtypeStruct((S, 2 * D), bf16),
        in_specs=[pl.BlockSpec(memory_space=pl.ANY)] * 10,
        out_specs=pl.BlockSpec(memory_space=pl.ANY),
        scratch_shapes=[
            vm((S, D), bf16), vm((DF, S), bf16), vm((DF, S), bf16), vm((S, D), bf16), vm((D, 3 * D), bf16),
            vm((D, D), bf16), vm((640, 256), bf16), vm((256, 640), bf16), vm((32, 128, 128), bf16),
            vm((32, 128, 128), bf16), vm((S, D), bf16), vm((S, D), bf16),
            vm((320, 256), u32), vm((128, 640), u32), vm((6, S, 128), f32), vm((4, 320, 128), f32),
            vm((6, 1024, 128), u32),
            vm((320, 1280), u32), vm((NB, 64, 640), u32), vm((320, 640), u32), vm((7, 128, 128), f32),
            vm((8, 128), i32), vm((NB, H, 16, 128), u32), vm((NB, H, 16, 128), u32), vm((NB, 64, 1024), u32),
            vm((NB, 64, 640), u32),
            pltpu.SemaphoreType.DMA((24,)), pltpu.SemaphoreType.DMA((2, NB)),
            vm((8 + 8 * CFG['pad'], 128), f32),
        ],
        compiler_params=pltpu.CompilerParams(vmem_limit_bytes=120 * 1024 * 1024),
        name="fused_kernel",
    )(A_x.reshape(S, D), A_w_r.T, A_w_i.T, B_x.reshape(S, D), B_wqkv, B_wo, mf, nf, g, hm)
    return out.reshape(1, S, 2 * D)
```

```python
import functools
import math

import jax
import jax.numpy as jnp
import numpy as np
import ml_dtypes
from jax.experimental import pallas as pl
from jax.experimental.pallas import tpu as pltpu

S = 2048
D = 640
DF = 321
H = 32
DH = 20
NB = 16
NEG = -1e30
SCALE = (DH ** -0.5) * 1.4426950408889634
bf16 = jnp.bfloat16
f32 = jnp.float32
u32 = jnp.uint32
i32 = jnp.int32
NT = (((1,), (1,)), ((), ()))
C1, C2 = math.cos(2 * math.pi / 5), math.cos(4 * math.pi / 5)
S1, S2 = math.sin(2 * math.pi / 5), math.sin(4 * math.pi / 5)


def _make_consts():
    l = np.arange(128)
    k1 = np.where(l < 64, 1 + 5 * l, 4 + 5 * (l - 64))
    k2 = np.where(l < 64, 2 + 5 * l, 3 + 5 * (l - 64))
    n = np.arange(128)[:, None]
    sig = np.where(l < 64, 1.0, -1.0)[None, :]

    def cs(k):
        th = 2 * np.pi * ((n * k[None, :]) % D) / D
        return np.cos(th), np.sin(th)

    ms = []
    for k in (k1, k2):
        c, s = cs(k)
        ms.append(np.block([[c, -s], [sig * s, sig * c]]))
    k0 = np.where(l <= 64, 5 * l, 5 * (l - 64))
    c, s = cs(k0)
    low = (l <= 64)[None, :]
    m0 = np.where(low, c, -s)
    ck0 = np.where((k0 == 0) | (k0 == 320), 1.0, 2.0)
    n0 = (m0 * ck0[None, :]).T / (S * D)
    mf = np.concatenate([np.concatenate(ms, axis=0),
                         np.concatenate([m0, np.zeros((128, 128))], axis=1)], axis=0)
    nf = np.concatenate([ms[0].T * (2.0 / (S * D)), ms[1].T * (2.0 / (S * D)),
                         np.concatenate([n0, np.zeros((128, 128))], axis=0)], axis=1)
    a1 = np.arange(32)[:, None, None]
    a2 = np.arange(64)[None, :, None]
    n2 = np.arange(64)[None, None, :]
    a = 2 * np.pi * ((n2 * (a1 + 32 * a2)) % S) / S
    gr, gi = np.cos(a), -np.sin(a)
    g = np.concatenate([np.concatenate([gr, -gi], axis=2), np.concatenate([gi, gr], axis=2)], axis=1)
    hm = np.transpose(g, (0, 2, 1))
    cvt = lambda z: np.ascontiguousarray(z).astype(ml_dtypes.bfloat16)
    return cvt(mf), cvt(nf), cvt(g), cvt(hm)


def pk(x):
    return pltpu.bitcast(x, u32)


def unpk(x):
    return pltpu.bitcast(x, bf16)


def _cmul(re, im, wr, wi):
    e = 1e-12
    if abs(wi) < e:
        if abs(wr - 1) < e:
            return re, im
        return re * wr, im * wr
    if abs(abs(wr) - abs(wi)) < e:
        if wi / wr > 0:
            return (re - im) * wr, (re + im) * wr
        return (re + im) * wr, (im - re) * wr
    return re * wr - im * wi, re * wi + im * wr


def _fft(xr, xi, sgn):
    n = len(xr)
    if n == 1:
        return xr, xi
    if n == 2:
        return [xr[0] + xr[1], xr[0] - xr[1]], [xi[0] + xi[1], xi[0] - xi[1]]
    er, ei = _fft(xr[0::2], xi[0::2], sgn)
    ar, ai = _fft(xr[1::4], xi[1::4], sgn)
    br, bi = _fft(xr[3::4], xi[3::4], sgn)
    outr = [None] * n
    outi = [None] * n
    q = n // 4
    for k in range(q):
        a1 = sgn * 2 * math.pi * k / n
        a3 = 3 * a1
        z1r, z1i = _cmul(ar[k], ai[k], math.cos(a1), math.sin(a1))
        z3r, z3i = _cmul(br[k], bi[k], math.cos(a3), math.sin(a3))
        sr, si = z1r + z3r, z1i + z3i
        dr, di = z1r - z3r, z1i - z3i
        outr[k], outi[k] = er[k] + sr, ei[k] + si
        outr[k + 2 * q], outi[k + 2 * q] = er[k] - sr, ei[k] - si
        if sgn < 0:
            outr[k + q], outi[k + q] = er[k + q] + di, ei[k + q] - dr
            outr[k + 3 * q], outi[k + 3 * q] = er[k + q] - di, ei[k + q] + dr
        else:
            outr[k + q], outi[k + q] = er[k + q] - di, ei[k + q] + dr
            outr[k + 3 * q], outi[k + 3 * q] = er[k + q] + di, ei[k + q] - dr
    return outr, outi


def _rcp(l):
    x = pl.reciprocal(l, approx=True)
    return x * (2.0 - l * x)


def _dot(a, b):
    return jnp.dot(a, b, preferred_element_type=f32)


def _kernel(xa_h, wrT_h, wiT_h, xb_h, wqkv_h, wo_h, mf_h, nf_h, g_h, h_h, out_h,
            xa_v, wrT_v, wiT_v, xb_v, wqkv_v, wo_v, mf_v, nf_v, g_v, h_v, oa_v, ob_v,
            mf_s, nf_s, u_s, st_s, wp_s,
            wqv_s, xb_s, wo_s, bias_s, z_s, wq_s, vw_s, kw_s, o_s,
            isem, osem):
    def cp(src, dst, k):
        return pltpu.make_async_copy(src, dst, isem.at[k])

    def rows(ref, c, n):
        return ref.at[pl.ds(c * n, n), :]

    d_mf = cp(mf_h, mf_v, 0)
    d_xa = [cp(rows(xa_h, c, 1024), rows(xa_v, c, 1024), 1 + c) for c in range(2)]
    d_wk = cp(wqkv_h.at[:, D:2 * D], wqkv_v.at[:, D:2 * D], 5)
    d_xb = [cp(xb_h.at[lo:hi, :], xb_v.at[lo:hi, :], 18 + c) for c, (lo, hi) in
            enumerate(((0, 256), (256, 768), (768, S)))]
    d_wq = cp(wqkv_h.at[:, 0:D], wqkv_v.at[:, 0:D], 10)
    d_wv = cp(wqkv_h.at[:, 2 * D:3 * D], wqkv_v.at[:, 2 * D:3 * D], 11)
    d_wr = [cp(wrT_h.at[:, c * 1024:(c + 1) * 1024], wrT_v.at[:, c * 1024:(c + 1) * 1024], 12 + 10 * c) for c in range(2)]
    d_wi = [cp(wiT_h.at[:, c * 1024:(c + 1) * 1024], wiT_v.at[:, c * 1024:(c + 1) * 1024], 13 + 10 * c) for c in range(2)]
    d_g = cp(g_h, g_v, 14)
    d_h = cp(h_h, h_v, 15)
    d_wo = cp(wo_h, wo_v, 16)
    d_nf = cp(nf_h, nf_v, 17)

    late = (d_g, d_h, d_wo, d_nf)
    for d in ([d_wk] + d_xb + [d_mf, d_xa[0], d_xa[1], d_wr[0], d_wi[0], d_wq, d_wv, d_wr[1], d_wi[1]]
              + list(late)):
        d.start()

    def p1_block(i):
        r0 = pl.multiple_of(i * 128, 128)
        xt = [xa_v[pl.ds(r0, 128), t * 128:(t + 1) * 128].astype(f32) for t in range(5)]
        t1, t2 = xt[1] + xt[4], xt[2] + xt[3]
        t3, t4 = xt[1] - xt[4], xt[2] - xt[3]
        y0 = (xt[0] + t1 + t2).astype(bf16)
        y1r = (xt[0] + C1 * t1 + C2 * t2).astype(bf16)
        y2r = (xt[0] + C2 * t1 + C1 * t2).astype(bf16)
        y1i = ((-S1) * t3 - S2 * t4).astype(bf16)
        y2i = ((-S2) * t3 + S1 * t4).astype(bf16)
        for p, (yr, yi) in enumerate(((y1r, y1i), (y2r, y2i))):
            for n in range(2):
                m_r = unpk(mf_s[p * 128:p * 128 + 64, n * 128:(n + 1) * 128])
                m_i = unpk(mf_s[p * 128 + 64:p * 128 + 128, n * 128:(n + 1) * 128])
                u_s[p + 3 * n, pl.ds(r0, 128), :] = _dot(yr, m_r) + _dot(yi, m_i)
        e = _dot(y0, unpk(mf_s[256:320, 0:128]))
        lane = jax.lax.broadcasted_iota(i32, (128, 128), 1)
        u_s[2, pl.ds(r0, 128), :] = e
        u_s[5, pl.ds(r0, 128), :] = jnp.where((lane & 63) == 0, 0.0, pltpu.roll(e, 64, 1))

    def fft_set(p, r, sgn, toks=None):
        off = pl.multiple_of(r * 8, 8)
        xr = [u_s[p, pl.ds(64 * n + off, 8), :] for n in range(32)]
        xi = [u_s[3 + p, pl.ds(64 * n + off, 8), :] for n in range(32)]
        if toks is not None:
            for n in range(16):
                tk = toks[0] if n % 2 == 0 else (toks[1] if n % 4 == 1 else toks[2])
                xr[n] = pltpu.bitcast(pltpu.bitcast(xr[n], i32) | tk, f32)
                xi[n] = pltpu.bitcast(pltpu.bitcast(xi[n], i32) | tk, f32)
        yr, yi = _fft(xr, xi, sgn)
        for n in range(32):
            u_s[p, pl.ds(64 * n + off, 8), :] = yr[n]
            u_s[3 + p, pl.ds(64 * n + off, 8), :] = yi[n]

    def wprep(T, tk):
        c0 = pl.multiple_of(T * 128, 128)
        q0 = pl.multiple_of(T * 64, 64)
        zer = jnp.zeros((56, 128), f32)
        sub = jax.lax.broadcasted_iota(i32, (8, 128), 0)
        for j, ref in enumerate((wrT_v, wiT_v)):
            wv = pk(ref[0:320, pl.ds(c0, 128)])
            wv = (wv.reshape(20, 8, 128) | pltpu.bitcast(tk[j], u32)[None]).reshape(160, 128)
            jj = j + 2 * (T % 2)
            st_s[jj, 0:320, :] = unpk(wv).astype(f32)
            last = jnp.broadcast_to(ref[320:321, pl.ds(c0, 128)].astype(f32), (8, 128))
            last = jnp.where(sub == 0, last, 0.0)
            sl = lambda a: st_s[jj, pl.ds(a, 64, stride=5), :]
            tiles = (jnp.concatenate([sl(1), sl(4)], axis=0),
                     jnp.concatenate([sl(2), sl(3)], axis=0),
                     jnp.concatenate([sl(0), last, zer], axis=0))
            for p in range(3):
                wp_s[3 * j + p, pl.ds(q0, 64), :] = pk(tiles[p].astype(bf16).T)

    def mid_pair(a):
        wv = [wp_s[t, pl.ds(a, 64, stride=16), :] for t in range(6)]
        for j in range(2):
            k1 = 2 * a + j
            r0 = pl.multiple_of(k1 * 64, 64)
            if j == 0:
                wf = [pltpu.bitcast(w << 16, f32) for w in wv]
            else:
                wf = [pltpu.bitcast(w & jnp.uint32(0xFFFF0000), f32) for w in wv]
            gk, hk = g_v[k1], h_v[k1]
            for p in range(3):
                y = jnp.concatenate([u_s[p, pl.ds(r0, 64), :], u_s[3 + p, pl.ds(r0, 64), :]], axis=0).astype(bf16)
                x = _dot(gk, y)
                xr, xi = x[0:64], x[64:128]
                wr, wi = wf[p], wf[3 + p]
                pp = jnp.concatenate([xr * wr - xi * wi, xr * wi + xi * wr], axis=0).astype(bf16)
                z = _dot(hk, pp)
                u_s[p, pl.ds(r0, 64), :] = z[0:64]
                u_s[3 + p, pl.ds(r0, 64), :] = z[64:128]

    def p5_block(i, tk=None):
        r0 = pl.multiple_of(i * 128, 128)
        z = [u_s[t, pl.ds(r0, 128), :] for t in range(6)]
        if tk is not None:
            z = [jnp.concatenate([pltpu.bitcast(pltpu.bitcast(a[0:8], i32) | tk, f32), a[8:128]], axis=0) for a in z]
        lane = jax.lax.broadcasted_iota(i32, (128, 128), 1)
        ze = jnp.where(lane <= 64, z[2], pltpu.roll(z[5], 64, 1)).astype(bf16)
        z = [a.astype(bf16) for a in z]

        def prod(p, c0):
            return (_dot(z[p], unpk(nf_s[0:64, c0:c0 + 128])) + _dot(z[3 + p], unpk(nf_s[64:128, c0:c0 + 128])))
        r1, i1 = prod(0, 0), prod(0, 128)
        r2, i2 = prod(1, 256), prod(1, 384)
        t0 = _dot(ze, unpk(nf_s[0:64, 512:640]))
        a1 = t0 + C1 * r1 + C2 * r2
        b1 = S1 * i1 + S2 * i2
        a2 = t0 + C2 * r1 + C1 * r2
        b2 = S2 * i1 - S1 * i2
        ys = (t0 + r1 + r2, a1 - b1, a2 - b2, a2 + b2, a1 + b1)
        for t in range(5):
            oa_v[pl.ds(r0, 128), t * 128:(t + 1) * 128] = ys[t].astype(bf16)
        pltpu.make_async_copy(oa_v.at[pl.ds(r0, 128), :], out_h.at[pl.ds(r0, 128), 0:D], osem.at[0, i]).start()

    def setup_misc():
        row = jax.lax.broadcasted_iota(i32, (128, 128), 0)
        lane = jax.lax.broadcasted_iota(i32, (128, 128), 1)
        bias_s[0] = jnp.where(row <= lane, 0.0, NEG).astype(f32)
        r5, q5 = row & 31, lane & 31
        grp, lg = row >> 5, lane >> 5
        bad5 = (((grp == 0) & (lg == 0) & (r5 > q5)) | ((grp == 1) & (lg == 3) & (r5 <= q5))
                | ((grp == 2) & (lg == 1) & (r5 > q5)) | ((grp == 3) & (lg == 2) & (r5 <= q5)))
        bias_s[1] = jnp.where(bad5, NEG, 0.0).astype(f32)
        bad6 = jnp.where(lg < 2, q5 - r5, r5 - q5 - 1) >= 0
        bias_s[2] = jnp.where(bad6, NEG, 0.0).astype(f32)
        z_s[...] = jnp.zeros(z_s.shape, i32)

    def proj_k(i):
        r0 = pl.multiple_of(i * 128, 128)
        xi = xb_v[pl.ds(r0, 128), :]
        xb_s[i] = pk(xi)
        tiles = []
        for n in range(5):
            acc = None
            for kt in range(5):
                r = _dot(xi[:, kt * 128:(kt + 1) * 128], wqkv_v[kt * 128:(kt + 1) * 128, D + n * 128:D + (n + 1) * 128])
                acc = r if acc is None else acc + r
            tiles.append(pk(acc.astype(bf16)))
        lane = jax.lax.broadcasted_iota(i32, (64, 128), 1)
        for g in range(8):
            off = (80 * g) % 128
            ta = (80 * g) // 128
            if off == 0:
                w = tiles[ta]
            else:
                w = pltpu.roll(tiles[ta], 128 - off, 1)
                if off + 80 > 128:
                    w = jnp.where(lane < 128 - off, w, pltpu.roll(tiles[ta + 1], 128 - off, 1))
            kw_s[i, :, g * 128:(g + 1) * 128] = w

    def proj_qv(i):
        xi = unpk(xb_s[i])
        toks = []
        zero = z_s[...]

        def part(c0):
            outs = []
            for n in range(5):
                acc = None
                for kt in range(5):
                    r = _dot(xi[:, kt * 128:(kt + 1) * 128],
                             unpk(wqv_s[kt * 64:(kt + 1) * 64, c0 + n * 128:c0 + (n + 1) * 128]))
                    if kt == 0:
                        toks.append(pltpu.bitcast(r[0:8], i32) & zero)
                    acc = r if acc is None else acc + r
                outs.append(acc)
            return outs
        sub = jax.lax.broadcasted_iota(i32, (16, 128), 0)
        qT = jnp.concatenate([pk((a * SCALE).astype(bf16).T) for a in part(0)], axis=0)
        for h in range(H):
            r0 = (20 * h) // 16 * 8
            dl = (20 * h) % 16 // 2
            wq_s[i, h] = jnp.where((sub >= dl) & (sub < dl + 10), qT[r0:r0 + 16], jnp.uint32(0))
        vT = jnp.concatenate([pk(a.astype(bf16).T) for a in part(D)], axis=0)
        one = jnp.uint32(0x3F803F80)
        for h in range(H):
            r0 = (20 * h) // 16 * 8
            dl = (20 * h) % 16 // 2
            if dl <= 2:
                w = jnp.concatenate([vT[r0:r0 + 8], jnp.where(sub[0:8] >= 4, one, vT[r0 + 8:r0 + 16])], axis=0)
            else:
                w = jnp.concatenate([jnp.where(sub[0:8] < 4, one, vT[r0:r0 + 8]), vT[r0 + 8:r0 + 16]], axis=0)
            vw_s[i, h] = w
        return toks

    def out_proj(i, tokz=None, tiles=(0, 1, 2, 3, 4)):
        r0 = pl.multiple_of(i * 128, 128)
        ot = [o_s[i, :, n * 128:(n + 1) * 128] for n in range(5)]
        if tokz is not None:
            ot = [(o.reshape(8, 8, 128) | pltpu.bitcast(tokz, u32)[None]).reshape(64, 128) for o in ot]
        ot = [unpk(o) for o in ot]
        for n in tiles:
            acc = None
            for kt in range(5):
                r = _dot(ot[kt], unpk(wo_s[kt * 64:(kt + 1) * 64, n * 128:(n + 1) * 128]))
                acc = r if acc is None else acc + r
            ob_v[pl.ds(r0, 128), n * 128:(n + 1) * 128] = acc.astype(bf16)
        if 4 in tiles:
            pltpu.make_async_copy(ob_v.at[pl.ds(r0, 128), :], out_h.at[pl.ds(r0, 128), D:2 * D], osem.at[1, i]).start()

    def attention(jobs, lag=4, drain=None):
        zero = z_s[...]
        seq = []
        info = []
        for jb, rounds in enumerate(jobs):
            nr = len(rounds)
            slots = sorted(set(r[3] for r in rounds))
            last = {s: max(t for t in range(nr) if rounds[t][3] == s) for s in slots}
            first = {s: min(t for t in range(nr) if rounds[t][3] == s) for s in slots}
            info.append((rounds, slots, first, last))
            for g in range(8):
                for t in range(nr):
                    seq.append((jb, g, t))

        def getw(qb, g, h):
            o = 20 * h - 80 * g
            r0 = o // 16 * 16
            parts = []
            if r0 > 0:
                parts.append(jnp.zeros((r0, 128), bf16))
            parts.append(unpk(wq_s[qb, h]))
            if 96 - r0 > 0:
                parts.append(jnp.zeros((96 - r0, 128), bf16))
            return jnp.concatenate(parts, axis=0)
        sv, mx, acc, tok, res = {}, {}, {}, {}, {}

        def qk(k):
            jb, g, t = seq[k]
            rounds, slots, first, last = info[jb]
            qb, kb, bi, sl = rounds[t]
            kk = unpk(kw_s[kb, :, g * 128:(g + 1) * 128])
            for j, h in enumerate(range(4 * g, 4 * g + 4)):
                key = (jb, sl, h)
                st = _dot(kk, getw(qb, g, h))
                tok[(k, j)] = pltpu.bitcast(st[0:8], i32) & zero
                if bi is not None:
                    st = st + bias_s[bi]
                sv[(k, j)] = st
                mm = jnp.max(st.reshape(16, 8, 128), axis=0)
                mx[key] = mm if t == first[sl] else jnp.maximum(mx[key], mm)
                if t == last[sl]:
                    mx[key] = jnp.broadcast_to(jnp.max(mx[key], axis=0, keepdims=True), (8, 128))

        def finish(jb):
            rounds, slots, first, last = info[jb]
            sub = jax.lax.broadcasted_iota(i32, (8, 128), 0)
            for sl in slots:
                qb = rounds[first[sl]][0]
                vregs = []
                for v in range(80):
                    h0, h1 = (8 * v) // 20, (8 * v + 7) // 20

                    def get(h):
                        r0 = (20 * h) // 16 * 16
                        return res[(jb, sl, h)][8 * v - r0:8 * v - r0 + 8]
                    vregs.append(get(h0) if h0 == h1 else jnp.where(sub < (20 * h1 - 8 * v), get(h0), get(h1)))
                oT = jnp.concatenate(vregs, axis=0).astype(bf16)
                for n in range(5):
                    o_s[qb, :, n * 128:(n + 1) * 128] = pk(oT[n * 128:(n + 1) * 128].T)

        def pv(k, kt):
            jb, g, t = seq[k]
            rounds, slots, first, last = info[jb]
            qb, kb, bi, sl = rounds[t]
            ptok = None
            for j, h in enumerate(range(4 * g, 4 * g + 4)):
                key = (jb, sl, h)
                m = mx[key]
                if kt is not None:
                    m = pltpu.bitcast(pltpu.bitcast(m, i32) | tok[(kt, j)], f32)
                s = sv.pop((k, j))
                p = jnp.exp2(s.reshape(16, 8, 128) - m[None]).reshape(128, 128).astype(bf16)
                r = _dot(unpk(vw_s[kb, h]), p)
                if j == 3:
                    ptok = pltpu.bitcast(pk(p)[56:64], i32) & zero
                acc[key] = r if t == first[sl] else acc[key] + r
                if t == last[sl]:
                    dl = 20 * h % 16
                    a = acc.pop(key)
                    l = a[24:32] if dl <= 4 else a[0:8]
                    res[key] = (a.reshape(4, 8, 128) * _rcp(l)[None]).reshape(32, 128)
            if g == 7 and t == len(rounds) - 1:
                finish(jb)
            return ptok
        nk = len(seq)
        for k in range(nk + lag):
            if k < nk:
                qk(k)
            if k - lag >= 0:
                kt = k - 1
                if kt >= nk or kt < 0:
                    kt = None
                pt = pv(k - lag, kt)
                if drain is not None and k - nk + 1 in drain and k >= nk:
                    drain[k - nk + 1](pt)
            if k == nk - 1 and drain is not None and 0 in drain:
                drain[0](tok[(nk - 1, 3)])

    def attention3(blocks, lag=4, drain=None):
        zero = z_s[...]
        zu = jnp.uint32(0)

        def lanes(n):
            return jax.lax.broadcasted_iota(i32, (n, 128), 1)
        seq = [(jb, g, t) for jb in range(len(blocks)) for g in range(8) for t in range(3)]
        zq = jnp.zeros((16, 128), bf16)

        def place(parts):
            out, pos = [], 0
            for r0, w in parts:
                out += [zq] * ((r0 - pos) // 16) + [unpk(w)]
                pos = r0 + 32
            out += [zq] * ((128 - pos) // 16)
            return jnp.concatenate(out, axis=0)

        def roll(x, a):
            return x if a % 128 == 0 else pltpu.roll(x, a % 128, 1)
        sv, pp, mx, acc, tok, res = {}, {}, {}, {}, {}, {}

        def qk(k):
            jb, g, t = seq[k]
            i = blocks[jb]
            cs = slice(g * 128, (g + 1) * 128)
            l16 = lanes(16)
            if t == 0:
                kk = unpk(kw_s[i - 1, :, cs])
            elif t == 1:
                kk = unpk(jnp.concatenate([kw_s[i, 0:16, cs], kw_s[i - 2, 48:64, cs]], axis=0))
                ka = kw_s[i - 2, 16:48, cs]
                kr = pltpu.roll(kw_s[i, 16:48, cs], 48, 1)
                km = [unpk(jnp.where(lanes(32) < 44, ka, kr)), unpk(jnp.where(lanes(32) < 84, ka, kr))]
            else:
                kc = [kw_s[i - 2, 0:16, cs], kw_s[i - 2, 16:32, cs], kw_s[i, 32:48, cs], kw_s[i, 48:64, cs]]
            for j, h in enumerate(range(4 * g, 4 * g + 4)):
                key = (jb, h)
                r0 = 20 * j // 16 * 16
                w32 = wq_s[i, h]
                if t == 0:
                    st = _dot(kk, place([(r0, w32)]))
                    tok[(k, j)] = pltpu.bitcast(st[0:8], i32) & zero
                elif t == 1:
                    def wsplit(thr):
                        return place([(r0, jnp.where(l16 < thr, w32, zu)), (r0 + 48, jnp.where(l16 >= thr, w32, zu))])
                    sp = _dot(kk, place([(r0, w32)]))
                    tok[(k, j)] = pltpu.bitcast(sp[0:8], i32) & zero
                    st = [sp + bias_s[1, 0:64], _dot(km[j // 2][0:32], wsplit(32)) + bias_s[1, 64:96],
                          _dot(km[j // 2][32:64], wsplit(96)) + bias_s[1, 96:128]]
                else:
                    c = roll(kc[3], 96 - r0)
                    for s in (2, 1, 0):
                        c = jnp.where(l16 < 32 * s + 32, roll(kc[s], 32 * s - r0), c)
                    w4 = place([(32 * s, jnp.where((l16 >> 5) == s, w32, zu)) for s in range(4)])
                    st = _dot(unpk(c), w4)
                    tok[(k, j)] = pltpu.bitcast(st[0:8], i32) & zero
                    st = st + bias_s[2, 0:32]
                if not isinstance(st, list):
                    st = [st]
                sv[(k, j)] = st
                mm = functools.reduce(jnp.maximum, [jnp.max(x.reshape(-1, 8, 128), axis=0) for x in st])
                mx[key] = mm if t == 0 else jnp.maximum(mx[key], mm)
                if t == 2:
                    mx[key] = jnp.broadcast_to(jnp.max(mx[key], axis=0, keepdims=True), (8, 128))

        def finish(jb):
            sub = jax.lax.broadcasted_iota(i32, (8, 128), 0)
            vregs = []
            for v in range(80):
                h0, h1 = (8 * v) // 20, (8 * v + 7) // 20

                def get(h):
                    r0 = (20 * h) // 16 * 16
                    return res[(jb, h)][8 * v - r0:8 * v - r0 + 8]
                vregs.append(get(h0) if h0 == h1 else jnp.where(sub < (20 * h1 - 8 * v), get(h0), get(h1)))
            oT = jnp.concatenate(vregs, axis=0).astype(bf16)
            for n in range(5):
                o_s[blocks[jb], :, n * 128:(n + 1) * 128] = pk(oT[n * 128:(n + 1) * 128].T)

        def pv(k, kt):
            jb, g, t = seq[k]
            i = blocks[jb]
            ptok = None
            l16 = lanes(16)
            for j, h in enumerate(range(4 * g, 4 * g + 4)):
                key = (jb, h)
                m = mx[key]
                if kt is not None:
                    m = pltpu.bitcast(pltpu.bitcast(m, i32) | tok[(kt, j)], f32)
                s = sv.pop((k, j))
                if t == 1:
                    s = [s[0][0:32], s[0][32:64], s[1], s[2]]
                ps = [jnp.exp2(x.reshape(-1, 8, 128) - m[None]).reshape(-1, 128) for x in s]
                if t == 0:
                    acc[key] = _dot(unpk(vw_s[i - 1, h]), ps[0].astype(bf16))
                elif t == 1:
                    pp[key] = ps
                else:
                    pc = ps[0]
                    d0, f3, m1, m2 = pp.pop(key)
                    l32 = lanes(32)
                    far = jnp.concatenate([jnp.where(l32 < 32, pc, 0.0),
                                           jnp.where(l32 < 32, m1, jnp.where(l32 < 64, pc, 0.0)),
                                           jnp.where(l32 < 96, m2, 0.0), f3], axis=0).astype(bf16)
                    dia = jnp.concatenate([d0, jnp.where(l32 >= 32, m1, 0.0),
                                           jnp.where(l32 >= 96, m2, jnp.where(l32 >= 64, pc, 0.0)),
                                           jnp.where(l32 >= 96, pc, 0.0)], axis=0).astype(bf16)
                    a = acc.pop(key) + _dot(unpk(vw_s[i - 2, h]), far) + _dot(unpk(vw_s[i, h]), dia)
                    dl = 20 * h % 16
                    l = a[24:32] if dl <= 4 else a[0:8]
                    res[key] = (a.reshape(4, 8, 128) * _rcp(l)[None]).reshape(32, 128)
                if j == 3:
                    ptok = pltpu.bitcast(ps[-1][24:32], i32) & zero
            if g == 7 and t == 2:
                finish(jb)
            return ptok
        nk = len(seq)
        assert drain is None or max(drain) <= lag
        for k in range(nk + lag):
            if k < nk:
                qk(k)
            if k - lag >= 0:
                kt = k - 1
                if kt >= nk or kt < 0:
                    kt = None
                pt = pv(k - lag, kt)
                if drain is not None and k - nk + 1 in drain and k != nk - 1:
                    drain[k - nk + 1](pt)
            if k == nk - 1 and drain is not None and 0 in drain:
                drain[0](tok[(k, 3)])

    def rep(fn, n, iters):
        per = n // iters

        def body(it, carry):
            for q in range(per):
                fn(per * it + q)
            return carry
        jax.lax.fori_loop(0, iters, body, 0)

    setup_misc()

    d_wk.wait()
    for j in range(NB):
        if j in (0, 2, 6):
            d_xb[(0, 2, 6).index(j)].wait()
        proj_k(j)

    d_mf.wait()
    d_xa[0].wait()
    d_xa[1].wait()
    d_wr[0].wait()
    d_wi[0].wait()
    mf_s[...] = pk(mf_v[...])
    for j in range(NB):
        p1_block(j)
    d_wq.wait()
    d_wv.wait()
    wqv_s[:, 0:D] = pk(wqkv_v[:, 0:D])
    wqv_s[:, D:2 * D] = pk(wqkv_v[:, 2 * D:3 * D])

    for q in range(8):
        if q == 4:
            d_wr[1].wait()
            d_wi[1].wait()
            for d in late:
                d.wait()
            wo_s[...] = pk(wo_v[...])
            nf_s[...] = pk(nf_v[...])
        tk = proj_qv(q)
        for j in range(3):
            fft_set(j, q, -1, tk[3 * j:3 * j + 3])
        wprep(2 * q, tk[1:3])
        wprep(2 * q + 1, tk[6:8])

    rep(mid_pair, 16, 2)

    for q in range(8):
        tk = proj_qv(8 + q)
        for j in range(3):
            fft_set(j, q, +1, tk[3 * j:3 * j + 3])

    attention([[(0, 0, 0, 0), (1, 0, None, 1), (1, 1, 0, 1)]], drain={0: lambda tz: p5_block(0, tz)})
    attention3(list(range(2, NB)),
               drain={0: lambda tz: out_proj(0, tz, (0, 1, 2)), 2: lambda tz: out_proj(0, tz, (3, 4)),
                      4: lambda tz: p5_block(1, tz)})

    def phase_g(u):
        p5_block(2 + u)
        out_proj(1 + u)
    rep(phase_g, NB - 2, 2)
    out_proj(NB - 1)

    def loop_f(i, carry):
        r0 = pl.multiple_of(i * 128, 128)
        pltpu.make_async_copy(oa_v.at[pl.ds(r0, 128), :], out_h.at[pl.ds(r0, 128), 0:D], osem.at[0, i]).wait()
        pltpu.make_async_copy(ob_v.at[pl.ds(r0, 128), :], out_h.at[pl.ds(r0, 128), D:2 * D], osem.at[1, i]).wait()
        return carry
    jax.lax.fori_loop(0, NB, loop_f, 0)


_CONSTS = _make_consts()


@jax.jit
def pallas_concat_heads__spectral_gfnet__sliding_block__prompt_kernel(A_x, A_w_r, A_w_i, B_x, B_wqkv, B_wo):
    mf, nf, g, hm = _CONSTS
    vm = pltpu.VMEM
    out = pl.pallas_call(
        _kernel,
        out_shape=jax.ShapeDtypeStruct((S, 2 * D), bf16),
        in_specs=[pl.BlockSpec(memory_space=pl.ANY)] * 10,
        out_specs=pl.BlockSpec(memory_space=pl.ANY),
        scratch_shapes=[
            vm((S, D), bf16), vm((DF, S), bf16), vm((DF, S), bf16), vm((S, D), bf16), vm((D, 3 * D), bf16),
            vm((D, D), bf16), vm((640, 256), bf16), vm((256, 640), bf16), vm((32, 128, 128), bf16),
            vm((32, 128, 128), bf16), vm((S, D), bf16), vm((S, D), bf16),
            vm((320, 256), u32), vm((128, 640), u32), vm((6, S, 128), f32), vm((4, 320, 128), f32),
            vm((6, 1024, 128), u32),
            vm((320, 1280), u32), vm((NB, 64, 640), u32), vm((320, 640), u32), vm((3, 128, 128), f32),
            vm((8, 128), i32), vm((NB, H, 16, 128), u32), vm((NB, H, 16, 128), u32), vm((NB, 64, 1024), u32),
            vm((NB, 64, 640), u32),
            pltpu.SemaphoreType.DMA((24,)), pltpu.SemaphoreType.DMA((2, NB)),
        ],
        compiler_params=pltpu.CompilerParams(vmem_limit_bytes=120 * 1024 * 1024),
        name="fused_kernel",
    )(A_x.reshape(S, D), A_w_r.T, A_w_i.T, B_x.reshape(S, D), B_wqkv, B_wo, mf, nf, g, hm)
    return out.reshape(1, S, 2 * D)
```

```python
import functools
import math

import jax
import jax.numpy as jnp
import numpy as np
import ml_dtypes
from jax.experimental import pallas as pl
from jax.experimental.pallas import tpu as pltpu

S = 2048
D = 640
DF = 321
H = 32
DH = 20
NB = 16
NEG = -1e30
SCALE = (DH ** -0.5) * 1.4426950408889634
bf16 = jnp.bfloat16
f32 = jnp.float32
u32 = jnp.uint32
i32 = jnp.int32
C1, C2 = math.cos(2 * math.pi / 5), math.cos(4 * math.pi / 5)
S1, S2 = math.sin(2 * math.pi / 5), math.sin(4 * math.pi / 5)


def _make_consts():
    l = np.arange(128)
    k1 = np.where(l < 64, 1 + 5 * l, 4 + 5 * (l - 64))
    k2 = np.where(l < 64, 2 + 5 * l, 3 + 5 * (l - 64))
    n = np.arange(128)[:, None]
    sig = np.where(l < 64, 1.0, -1.0)[None, :]

    def cs(k):
        th = 2 * np.pi * ((n * k[None, :]) % D) / D
        return np.cos(th), np.sin(th)

    ms = []
    for k in (k1, k2):
        c, s = cs(k)
        ms.append(np.block([[c, -s], [sig * s, sig * c]]))
    k0 = np.where(l <= 64, 5 * l, 5 * (l - 64))
    c, s = cs(k0)
    low = (l <= 64)[None, :]
    m0 = np.where(low, c, -s)
    ck0 = np.where((k0 == 0) | (k0 == 320), 1.0, 2.0)
    n0 = (m0 * ck0[None, :]).T / (S * D)
    mf = np.concatenate([np.concatenate(ms, axis=0),
                         np.concatenate([m0, np.zeros((128, 128))], axis=1)], axis=0)
    nf = np.concatenate([ms[0].T * (2.0 / (S * D)), ms[1].T * (2.0 / (S * D)),
                         np.concatenate([n0, np.zeros((128, 128))], axis=0)], axis=1)
    a1 = np.arange(32)[:, None, None]
    a2 = np.arange(64)[None, :, None]
    n2 = np.arange(64)[None, None, :]
    a = 2 * np.pi * ((n2 * (a1 + 32 * a2)) % S) / S
    gr, gi = np.cos(a), -np.sin(a)
    g = np.concatenate([np.concatenate([gr, -gi], axis=2), np.concatenate([gi, gr], axis=2)], axis=1)
    hm = np.transpose(g, (0, 2, 1))
    cvt = lambda z: np.ascontiguousarray(z).astype(ml_dtypes.bfloat16)
    return cvt(mf), cvt(nf), cvt(g), cvt(hm)


def pk(x):
    return pltpu.bitcast(x, u32)


def unpk(x):
    return pltpu.bitcast(x, bf16)


def _cmul(re, im, wr, wi):
    e = 1e-12
    if abs(wi) < e:
        if abs(wr - 1) < e:
            return re, im
        return re * wr, im * wr
    if abs(abs(wr) - abs(wi)) < e:
        if wi / wr > 0:
            return (re - im) * wr, (re + im) * wr
        return (re + im) * wr, (im - re) * wr
    return re * wr - im * wi, re * wi + im * wr


def _fft(xr, xi, sgn):
    n = len(xr)
    if n == 1:
        return xr, xi
    if n == 2:
        return [xr[0] + xr[1], xr[0] - xr[1]], [xi[0] + xi[1], xi[0] - xi[1]]
    er, ei = _fft(xr[0::2], xi[0::2], sgn)
    ar, ai = _fft(xr[1::4], xi[1::4], sgn)
    br, bi = _fft(xr[3::4], xi[3::4], sgn)
    outr = [None] * n
    outi = [None] * n
    q = n // 4
    for k in range(q):
        a1 = sgn * 2 * math.pi * k / n
        a3 = 3 * a1
        z1r, z1i = _cmul(ar[k], ai[k], math.cos(a1), math.sin(a1))
        z3r, z3i = _cmul(br[k], bi[k], math.cos(a3), math.sin(a3))
        sr, si = z1r + z3r, z1i + z3i
        dr, di = z1r - z3r, z1i - z3i
        outr[k], outi[k] = er[k] + sr, ei[k] + si
        outr[k + 2 * q], outi[k + 2 * q] = er[k] - sr, ei[k] - si
        if sgn < 0:
            outr[k + q], outi[k + q] = er[k + q] + di, ei[k + q] - dr
            outr[k + 3 * q], outi[k + 3 * q] = er[k + q] - di, ei[k + q] + dr
        else:
            outr[k + q], outi[k + q] = er[k + q] - di, ei[k + q] + dr
            outr[k + 3 * q], outi[k + 3 * q] = er[k + q] + di, ei[k + q] - dr
    return outr, outi


def _rcp(l):
    x = pl.reciprocal(l, approx=True)
    return x * (2.0 - l * x)


def _dot(a, b):
    return jnp.dot(a, b, preferred_element_type=f32)


def _kernel(xa_h, wrT_h, wiT_h, xb_h, wqkv_h, wo_h, mf_h, nf_h, g_h, h_h, out_h,
            xa_v, wrT_v, wiT_v, xb_v, wqkv_v, wo_v, mf_v, nf_v, g_v, h_v, oa_v, ob_v,
            mf_s, nf_s, u_s, st_s, wp_s,
            wqv_s, xb_s, wo_s, bias_s, z_s, wq_s, vw_s, kw_s, o_s,
            isem, osem, tsem):
    def cp(src, dst, k):
        return pltpu.make_async_copy(src, dst, isem.at[k])

    def rows(ref, c, n):
        return ref.at[pl.ds(c * n, n), :]

    d_mf = cp(mf_h, mf_v, 0)
    d_xa = [cp(rows(xa_h, c, 1024), rows(xa_v, c, 1024), 1 + c) for c in range(2)]
    d_wk = cp(wqkv_h.at[:, D:2 * D], wqkv_v.at[:, D:2 * D], 5)
    d_xb = [cp(xb_h.at[lo:hi, :], xb_v.at[lo:hi, :], 18 + c) for c, (lo, hi) in
            enumerate(((0, 256), (256, 768), (768, S)))]
    d_wq = cp(wqkv_h.at[:, 0:D], wqkv_v.at[:, 0:D], 10)
    d_wv = cp(wqkv_h.at[:, 2 * D:3 * D], wqkv_v.at[:, 2 * D:3 * D], 11)
    d_wr = [cp(wrT_h.at[:, c * 1024:(c + 1) * 1024], wrT_v.at[:, c * 1024:(c + 1) * 1024], 12 + 10 * c) for c in range(2)]
    d_wi = [cp(wiT_h.at[:, c * 1024:(c + 1) * 1024], wiT_v.at[:, c * 1024:(c + 1) * 1024], 13 + 10 * c) for c in range(2)]
    d_g = cp(g_h, g_v, 14)
    d_h = cp(h_h, h_v, 15)
    d_wo = cp(wo_h, wo_v, 16)
    d_nf = cp(nf_h, nf_v, 17)

    late = (d_g, d_h, d_wo, d_nf)
    for d in ([d_wk] + d_xb + [d_mf, d_xa[0], d_xa[1], d_wr[0], d_wi[0], d_wq, d_wv, d_wr[1], d_wi[1]]
              + list(late)):
        d.start()

    def p1_block(i):
        r0 = pl.multiple_of(i * 128, 128)
        xt = [xa_v[pl.ds(r0, 128), t * 128:(t + 1) * 128].astype(f32) for t in range(5)]
        t1, t2 = xt[1] + xt[4], xt[2] + xt[3]
        t3, t4 = xt[1] - xt[4], xt[2] - xt[3]
        y0 = (xt[0] + t1 + t2).astype(bf16)
        y1r = (xt[0] + C1 * t1 + C2 * t2).astype(bf16)
        y2r = (xt[0] + C2 * t1 + C1 * t2).astype(bf16)
        y1i = ((-S1) * t3 - S2 * t4).astype(bf16)
        y2i = ((-S2) * t3 + S1 * t4).astype(bf16)
        for p, (yr, yi) in enumerate(((y1r, y1i), (y2r, y2i))):
            for n in range(2):
                m_r = unpk(mf_s[p * 128:p * 128 + 64, n * 128:(n + 1) * 128])
                m_i = unpk(mf_s[p * 128 + 64:p * 128 + 128, n * 128:(n + 1) * 128])
                u_s[p + 3 * n, pl.ds(r0, 128), :] = _dot(yr, m_r) + _dot(yi, m_i)
        e = _dot(y0, unpk(mf_s[256:320, 0:128]))
        lane = jax.lax.broadcasted_iota(i32, (128, 128), 1)
        u_s[2, pl.ds(r0, 128), :] = e
        u_s[5, pl.ds(r0, 128), :] = jnp.where((lane & 63) == 0, 0.0, pltpu.roll(e, 64, 1))

    def fft_set(p, r, sgn, toks=None):
        off = pl.multiple_of(r * 8, 8)
        xr = [u_s[p, pl.ds(64 * n + off, 8), :] for n in range(32)]
        xi = [u_s[3 + p, pl.ds(64 * n + off, 8), :] for n in range(32)]
        if toks is not None:
            for n in range(16):
                tk = toks[0] if n % 2 == 0 else (toks[1] if n % 4 == 1 else toks[2])
                xr[n] = pltpu.bitcast(pltpu.bitcast(xr[n], i32) | tk, f32)
                xi[n] = pltpu.bitcast(pltpu.bitcast(xi[n], i32) | tk, f32)
        yr, yi = _fft(xr, xi, sgn)
        for n in range(32):
            u_s[p, pl.ds(64 * n + off, 8), :] = yr[n]
            u_s[3 + p, pl.ds(64 * n + off, 8), :] = yi[n]

    def wprep(T, tk):
        c0 = pl.multiple_of(T * 128, 128)
        q0 = pl.multiple_of(T * 64, 64)
        zer = jnp.zeros((56, 128), f32)
        sub = jax.lax.broadcasted_iota(i32, (8, 128), 0)
        for j, ref in enumerate((wrT_v, wiT_v)):
            wv = pk(ref[0:320, pl.ds(c0, 128)])
            wv = (wv.reshape(20, 8, 128) | pltpu.bitcast(tk[j], u32)[None]).reshape(160, 128)
            jj = j + 2 * (T % 2)
            st_s[jj, 0:320, :] = unpk(wv).astype(f32)
            last = jnp.broadcast_to(ref[320:321, pl.ds(c0, 128)].astype(f32), (8, 128))
            last = jnp.where(sub == 0, last, 0.0)
            sl = lambda a: st_s[jj, pl.ds(a, 64, stride=5), :]
            tiles = (jnp.concatenate([sl(1), sl(4)], axis=0),
                     jnp.concatenate([sl(2), sl(3)], axis=0),
                     jnp.concatenate([sl(0), last, zer], axis=0))
            for p in range(3):
                wp_s[3 * j + p, pl.ds(q0, 64), :] = pk(tiles[p].astype(bf16).T)

    def mid_pair(a):
        wv = [wp_s[t, pl.ds(a, 64, stride=16), :] for t in range(6)]
        for j in range(2):
            k1 = 2 * a + j
            r0 = pl.multiple_of(k1 * 64, 64)
            if j == 0:
                wf = [pltpu.bitcast(w << 16, f32) for w in wv]
            else:
                wf = [pltpu.bitcast(w & jnp.uint32(0xFFFF0000), f32) for w in wv]
            gk, hk = g_v[k1], h_v[k1]
            for p in range(3):
                y = jnp.concatenate([u_s[p, pl.ds(r0, 64), :], u_s[3 + p, pl.ds(r0, 64), :]], axis=0).astype(bf16)
                x = _dot(gk, y)
                xr, xi = x[0:64], x[64:128]
                wr, wi = wf[p], wf[3 + p]
                pp = jnp.concatenate([xr * wr - xi * wi, xr * wi + xi * wr], axis=0).astype(bf16)
                z = _dot(hk, pp)
                u_s[p, pl.ds(r0, 64), :] = z[0:64]
                u_s[3 + p, pl.ds(r0, 64), :] = z[64:128]

    def p5_block(i, tk=None):
        r0 = pl.multiple_of(i * 128, 128)
        z = [u_s[t, pl.ds(r0, 128), :] for t in range(6)]
        if tk is not None:
            z = [jnp.concatenate([pltpu.bitcast(pltpu.bitcast(a[0:8], i32) | tk, f32), a[8:128]], axis=0) for a in z]
        lane = jax.lax.broadcasted_iota(i32, (128, 128), 1)
        ze = jnp.where(lane <= 64, z[2], pltpu.roll(z[5], 64, 1)).astype(bf16)
        z = [a.astype(bf16) for a in z]

        def prod(p, c0):
            return (_dot(z[p], unpk(nf_s[0:64, c0:c0 + 128])) + _dot(z[3 + p], unpk(nf_s[64:128, c0:c0 + 128])))
        r1, i1 = prod(0, 0), prod(0, 128)
        r2, i2 = prod(1, 256), prod(1, 384)
        t0 = _dot(ze, unpk(nf_s[0:64, 512:640]))
        a1 = t0 + C1 * r1 + C2 * r2
        b1 = S1 * i1 + S2 * i2
        a2 = t0 + C2 * r1 + C1 * r2
        b2 = S2 * i1 - S1 * i2
        ys = (t0 + r1 + r2, a1 - b1, a2 - b2, a2 + b2, a1 + b1)
        for t in range(5):
            oa_v[pl.ds(r0, 128), t * 128:(t + 1) * 128] = ys[t].astype(bf16)
        pltpu.make_async_copy(oa_v.at[pl.ds(r0, 128), :], out_h.at[pl.ds(r0, 128), 0:D], osem.at[0, i]).start()

    def setup_misc():
        row = jax.lax.broadcasted_iota(i32, (128, 128), 0)
        lane = jax.lax.broadcasted_iota(i32, (128, 128), 1)
        bias_s[0] = jnp.where(row <= lane, 0.0, NEG).astype(f32)
        r5, q5 = row & 31, lane & 31
        grp, lg = row >> 5, lane >> 5
        bad5 = (((grp == 0) & (lg == 0) & (r5 > q5)) | ((grp == 1) & (lg == 3) & (r5 <= q5))
                | ((grp == 2) & (lg == 1) & (r5 > q5)) | ((grp == 3) & (lg == 2) & (r5 <= q5)))
        bias_s[1] = jnp.where(bad5, NEG, 0.0).astype(f32)
        bad6 = jnp.where(lg < 2, q5 - r5, r5 - q5 - 1) >= 0
        bias_s[2] = jnp.where(bad6, NEG, 0.0).astype(f32)
        z_s[...] = jnp.zeros(z_s.shape, i32)

    def proj_k(i):
        r0 = pl.multiple_of(i * 128, 128)
        xi = xb_v[pl.ds(r0, 128), :]
        xb_s[i] = pk(xi)
        tiles = []
        for n in range(5):
            acc = None
            for kt in range(5):
                r = _dot(xi[:, kt * 128:(kt + 1) * 128], wqkv_v[kt * 128:(kt + 1) * 128, D + n * 128:D + (n + 1) * 128])
                acc = r if acc is None else acc + r
            tiles.append(pk(acc.astype(bf16)))
        lane = jax.lax.broadcasted_iota(i32, (64, 128), 1)
        for g in range(8):
            off = (80 * g) % 128
            ta = (80 * g) // 128
            if off == 0:
                w = tiles[ta]
            else:
                w = pltpu.roll(tiles[ta], 128 - off, 1)
                if off + 80 > 128:
                    w = jnp.where(lane < 128 - off, w, pltpu.roll(tiles[ta + 1], 128 - off, 1))
            kw_s[i, :, g * 128:(g + 1) * 128] = w

    def proj_qv(i):
        xi = unpk(xb_s[i])
        toks = []
        zero = z_s[...]

        def part(c0):
            outs = []
            for n in range(5):
                acc = None
                for kt in range(5):
                    r = _dot(xi[:, kt * 128:(kt + 1) * 128],
                             unpk(wqv_s[kt * 64:(kt + 1) * 64, c0 + n * 128:c0 + (n + 1) * 128]))
                    if kt == 0:
                        toks.append(pltpu.bitcast(r[0:8], i32) & zero)
                    acc = r if acc is None else acc + r
                outs.append(acc)
            return outs
        sub = jax.lax.broadcasted_iota(i32, (16, 128), 0)
        qT = jnp.concatenate([pk((a * SCALE).astype(bf16).T) for a in part(0)], axis=0)
        for h in range(H):
            r0 = (20 * h) // 16 * 8
            dl = (20 * h) % 16 // 2
            wq_s[i, h] = jnp.where((sub >= dl) & (sub < dl + 10), qT[r0:r0 + 16], jnp.uint32(0))
        vT = jnp.concatenate([pk(a.astype(bf16).T) for a in part(D)], axis=0)
        one = jnp.uint32(0x3F803F80)
        for h in range(H):
            r0 = (20 * h) // 16 * 8
            dl = (20 * h) % 16 // 2
            if dl <= 2:
                w = jnp.concatenate([vT[r0:r0 + 8], jnp.where(sub[0:8] >= 4, one, vT[r0 + 8:r0 + 16])], axis=0)
            else:
                w = jnp.concatenate([jnp.where(sub[0:8] < 4, one, vT[r0:r0 + 8]), vT[r0 + 8:r0 + 16]], axis=0)
            vw_s[i, h] = w
        return toks

    def last_copy(n):
        return pltpu.make_async_copy(ob_v.at[S - 128:S, n * 128:(n + 1) * 128],
                                     out_h.at[S - 128:S, D + n * 128:D + (n + 1) * 128], tsem.at[n])

    def out_proj(i, tokz=None, tiles=(0, 1, 2, 3, 4), split=False):
        r0 = pl.multiple_of(i * 128, 128)
        ot = [o_s[i, :, n * 128:(n + 1) * 128] for n in range(5)]
        if tokz is not None:
            ot = [(o.reshape(8, 8, 128) | pltpu.bitcast(tokz, u32)[None]).reshape(64, 128) for o in ot]
        ot = [unpk(o) for o in ot]
        for n in tiles:
            acc = None
            for kt in range(5):
                r = _dot(ot[kt], unpk(wo_s[kt * 64:(kt + 1) * 64, n * 128:(n + 1) * 128]))
                acc = r if acc is None else acc + r
            ob_v[pl.ds(r0, 128), n * 128:(n + 1) * 128] = acc.astype(bf16)
            if split:
                last_copy(n).start()
        if 4 in tiles and not split:
            pltpu.make_async_copy(ob_v.at[pl.ds(r0, 128), :], out_h.at[pl.ds(r0, 128), D:2 * D], osem.at[1, i]).start()

    def attention(jobs, lag=4, drain=None):
        zero = z_s[...]
        seq = []
        info = []
        for jb, rounds in enumerate(jobs):
            nr = len(rounds)
            slots = sorted(set(r[3] for r in rounds))
            last = {s: max(t for t in range(nr) if rounds[t][3] == s) for s in slots}
            first = {s: min(t for t in range(nr) if rounds[t][3] == s) for s in slots}
            info.append((rounds, slots, first, last))
            for g in range(8):
                for t in range(nr):
                    seq.append((jb, g, t))

        def getw(qb, g, h):
            o = 20 * h - 80 * g
            r0 = o // 16 * 16
            parts = []
            if r0 > 0:
                parts.append(jnp.zeros((r0, 128), bf16))
            parts.append(unpk(wq_s[qb, h]))
            if 96 - r0 > 0:
                parts.append(jnp.zeros((96 - r0, 128), bf16))
            return jnp.concatenate(parts, axis=0)
        sv, mx, acc, tok, res = {}, {}, {}, {}, {}

        def qk(k):
            jb, g, t = seq[k]
            rounds, slots, first, last = info[jb]
            qb, kb, bi, sl = rounds[t]
            kk = unpk(kw_s[kb, :, g * 128:(g + 1) * 128])
            for j, h in enumerate(range(4 * g, 4 * g + 4)):
                key = (jb, sl, h)
                st = _dot(kk, getw(qb, g, h))
                tok[(k, j)] = pltpu.bitcast(st[0:8], i32) & zero
                if bi is not None:
                    st = st + bias_s[bi]
                sv[(k, j)] = st
                mm = jnp.max(st.reshape(16, 8, 128), axis=0)
                mx[key] = mm if t == first[sl] else jnp.maximum(mx[key], mm)
                if t == last[sl]:
                    mx[key] = jnp.broadcast_to(jnp.max(mx[key], axis=0, keepdims=True), (8, 128))

        def finish(jb):
            rounds, slots, first, last = info[jb]
            sub = jax.lax.broadcasted_iota(i32, (8, 128), 0)
            for sl in slots:
                qb = rounds[first[sl]][0]
                vregs = []
                for v in range(80):
                    h0, h1 = (8 * v) // 20, (8 * v + 7) // 20

                    def get(h):
                        r0 = (20 * h) // 16 * 16
                        return res[(jb, sl, h)][8 * v - r0:8 * v - r0 + 8]
                    vregs.append(get(h0) if h0 == h1 else jnp.where(sub < (20 * h1 - 8 * v), get(h0), get(h1)))
                oT = jnp.concatenate(vregs, axis=0).astype(bf16)
                for n in range(5):
                    o_s[qb, :, n * 128:(n + 1) * 128] = pk(oT[n * 128:(n + 1) * 128].T)

        def pv(k, kt):
            jb, g, t = seq[k]
            rounds, slots, first, last = info[jb]
            qb, kb, bi, sl = rounds[t]
            ptok = None
            for j, h in enumerate(range(4 * g, 4 * g + 4)):
                key = (jb, sl, h)
                m = mx[key]
                if kt is not None:
                    m = pltpu.bitcast(pltpu.bitcast(m, i32) | tok[(kt, j)], f32)
                s = sv.pop((k, j))
                p = jnp.exp2(s.reshape(16, 8, 128) - m[None]).reshape(128, 128).astype(bf16)
                r = _dot(unpk(vw_s[kb, h]), p)
                if j == 3:
                    ptok = pltpu.bitcast(pk(p)[56:64], i32) & zero
                acc[key] = r if t == first[sl] else acc[key] + r
                if t == last[sl]:
                    dl = 20 * h % 16
                    a = acc.pop(key)
                    l = a[24:32] if dl <= 4 else a[0:8]
                    res[key] = (a.reshape(4, 8, 128) * _rcp(l)[None]).reshape(32, 128)
            if g == 7 and t == len(rounds) - 1:
                finish(jb)
            return ptok
        nk = len(seq)
        for k in range(nk + lag):
            if k < nk:
                qk(k)
            if k - lag >= 0:
                kt = k - 1
                if kt >= nk or kt < 0:
                    kt = None
                pt = pv(k - lag, kt)
                if drain is not None and k - nk + 1 in drain and k >= nk:
                    drain[k - nk + 1](pt)
            if k == nk - 1 and drain is not None and 0 in drain:
                drain[0](tok[(nk - 1, 3)])

    def attention3(blocks, lag=4, drain=None):
        zero = z_s[...]
        zu = jnp.uint32(0)

        def lanes(n):
            return jax.lax.broadcasted_iota(i32, (n, 128), 1)
        seq = [(jb, g, t) for jb in range(len(blocks)) for g in range(8) for t in range(3)]
        zq = jnp.zeros((16, 128), bf16)

        def place(parts):
            out, pos = [], 0
            for r0, w in parts:
                out += [zq] * ((r0 - pos) // 16) + [unpk(w)]
                pos = r0 + 32
            out += [zq] * ((128 - pos) // 16)
            return jnp.concatenate(out, axis=0)

        def roll(x, a):
            return x if a % 128 == 0 else pltpu.roll(x, a % 128, 1)
        sv, pp, mx, acc, tok, res = {}, {}, {}, {}, {}, {}

        def qk(k):
            jb, g, t = seq[k]
            i = blocks[jb]
            cs = slice(g * 128, (g + 1) * 128)
            l16 = lanes(16)
            if t == 0:
                kk = unpk(kw_s[i - 1, :, cs])
            elif t == 1:
                kk = unpk(jnp.concatenate([kw_s[i, 0:16, cs], kw_s[i - 2, 48:64, cs]], axis=0))
                ka = kw_s[i - 2, 16:48, cs]
                kr = pltpu.roll(kw_s[i, 16:48, cs], 48, 1)
                km = [unpk(jnp.where(lanes(32) < 44, ka, kr)), unpk(jnp.where(lanes(32) < 84, ka, kr))]
            else:
                kc = [kw_s[i - 2, 0:16, cs], kw_s[i - 2, 16:32, cs], kw_s[i, 32:48, cs], kw_s[i, 48:64, cs]]
            for j, h in enumerate(range(4 * g, 4 * g + 4)):
                key = (jb, h)
                r0 = 20 * j // 16 * 16
                w32 = wq_s[i, h]
                if t == 0:
                    st = _dot(kk, place([(r0, w32)]))
                    tok[(k, j)] = pltpu.bitcast(st[0:8], i32) & zero
                elif t == 1:
                    def wsplit(thr):
                        return place([(r0, jnp.where(l16 < thr, w32, zu)), (r0 + 48, jnp.where(l16 >= thr, w32, zu))])
                    sp = _dot(kk, place([(r0, w32)]))
                    tok[(k, j)] = pltpu.bitcast(sp[0:8], i32) & zero
                    st = [sp + bias_s[1, 0:64], _dot(km[j // 2][0:32], wsplit(32)) + bias_s[1, 64:96],
                          _dot(km[j // 2][32:64], wsplit(96)) + bias_s[1, 96:128]]
                else:
                    c = roll(kc[3], 96 - r0)
                    for s in (2, 1, 0):
                        c = jnp.where(l16 < 32 * s + 32, roll(kc[s], 32 * s - r0), c)
                    w4 = place([(32 * s, jnp.where((l16 >> 5) == s, w32, zu)) for s in range(4)])
                    st = _dot(unpk(c), w4)
                    tok[(k, j)] = pltpu.bitcast(st[0:8], i32) & zero
                    st = st + bias_s[2, 0:32]
                if not isinstance(st, list):
                    st = [st]
                sv[(k, j)] = st
                mm = functools.reduce(jnp.maximum, [jnp.max(x.reshape(-1, 8, 128), axis=0) for x in st])
                mx[key] = mm if t == 0 else jnp.maximum(mx[key], mm)
                if t == 2:
                    mx[key] = jnp.broadcast_to(jnp.max(mx[key], axis=0, keepdims=True), (8, 128))

        def finish(jb):
            sub = jax.lax.broadcasted_iota(i32, (8, 128), 0)
            vregs = []
            for v in range(80):
                h0, h1 = (8 * v) // 20, (8 * v + 7) // 20

                def get(h):
                    r0 = (20 * h) // 16 * 16
                    return res[(jb, h)][8 * v - r0:8 * v - r0 + 8]
                vregs.append(get(h0) if h0 == h1 else jnp.where(sub < (20 * h1 - 8 * v), get(h0), get(h1)))
            oT = jnp.concatenate(vregs, axis=0).astype(bf16)
            for n in range(5):
                o_s[blocks[jb], :, n * 128:(n + 1) * 128] = pk(oT[n * 128:(n + 1) * 128].T)

        def pv(k, kt):
            jb, g, t = seq[k]
            i = blocks[jb]
            ptok = None
            l16 = lanes(16)
            for j, h in enumerate(range(4 * g, 4 * g + 4)):
                key = (jb, h)
                m = mx[key]
                if kt is not None:
                    m = pltpu.bitcast(pltpu.bitcast(m, i32) | tok[(kt, j)], f32)
                s = sv.pop((k, j))
                if t == 1:
                    s = [s[0][0:32], s[0][32:64], s[1], s[2]]
                ps = [jnp.exp2(x.reshape(-1, 8, 128) - m[None]).reshape(-1, 128) for x in s]
                if t == 0:
                    acc[key] = _dot(unpk(vw_s[i - 1, h]), ps[0].astype(bf16))
                elif t == 1:
                    pp[key] = ps
                else:
                    pc = ps[0]
                    d0, f3, m1, m2 = pp.pop(key)
                    l32 = lanes(32)
                    far = jnp.concatenate([jnp.where(l32 < 32, pc, 0.0),
                                           jnp.where(l32 < 32, m1, jnp.where(l32 < 64, pc, 0.0)),
                                           jnp.where(l32 < 96, m2, 0.0), f3], axis=0).astype(bf16)
                    dia = jnp.concatenate([d0, jnp.where(l32 >= 32, m1, 0.0),
                                           jnp.where(l32 >= 96, m2, jnp.where(l32 >= 64, pc, 0.0)),
                                           jnp.where(l32 >= 96, pc, 0.0)], axis=0).astype(bf16)
                    a = acc.pop(key) + _dot(unpk(vw_s[i - 2, h]), far) + _dot(unpk(vw_s[i, h]), dia)
                    dl = 20 * h % 16
                    l = a[24:32] if dl <= 4 else a[0:8]
                    res[key] = (a.reshape(4, 8, 128) * _rcp(l)[None]).reshape(32, 128)
                if j == 3:
                    ptok = pltpu.bitcast(ps[-1][24:32], i32) & zero
            if g == 7 and t == 2:
                finish(jb)
            return ptok
        nk = len(seq)
        assert drain is None or max(drain) <= lag
        for k in range(nk + lag):
            if k < nk:
                qk(k)
            if k - lag >= 0:
                kt = k - (2 if seq[k - lag][2] == 2 else 1)
                if kt >= nk or kt < 0:
                    kt = None
                pt = pv(k - lag, kt)
                if drain is not None and k - nk + 1 in drain and k != nk - 1:
                    drain[k - nk + 1](pt)
            if k == nk - 1 and drain is not None and 0 in drain:
                drain[0](tok[(k, 3)])

    def rep(fn, n, iters):
        per = n // iters

        def body(it, carry):
            for q in range(per):
                fn(per * it + q)
            return carry
        jax.lax.fori_loop(0, iters, body, 0)

    setup_misc()

    d_wk.wait()
    for j in range(NB):
        if j in (0, 2, 6):
            d_xb[(0, 2, 6).index(j)].wait()
        proj_k(j)

    d_mf.wait()
    d_xa[0].wait()
    d_xa[1].wait()
    d_wr[0].wait()
    d_wi[0].wait()
    mf_s[...] = pk(mf_v[...])
    for j in range(NB):
        p1_block(j)
    d_wq.wait()
    d_wv.wait()
    wqv_s[:, 0:D] = pk(wqkv_v[:, 0:D])
    wqv_s[:, D:2 * D] = pk(wqkv_v[:, 2 * D:3 * D])

    for q in range(8):
        if q == 4:
            d_wr[1].wait()
            d_wi[1].wait()
            for d in late:
                d.wait()
            wo_s[...] = pk(wo_v[...])
            nf_s[...] = pk(nf_v[...])
        tk = proj_qv(q)
        for j in range(3):
            fft_set(j, q, -1, tk[3 * j:3 * j + 3])
        wprep(2 * q, tk[1:3])
        wprep(2 * q + 1, tk[6:8])

    def cut():
        def _body(it, carry):
            st_s[0, pl.ds(pl.multiple_of(it * 8, 8), 8), :] = jnp.zeros((8, 128), f32)
            return carry
        jax.lax.fori_loop(0, 2, _body, 0)
    cut()
    for a in range(16):
        mid_pair(a)
    cut()

    for q in range(8):
        tk = proj_qv(8 + q)
        for j in range(3):
            fft_set(j, q, +1, tk[3 * j:3 * j + 3])

    attention([[(0, 0, 0, 0), (1, 0, None, 1), (1, 1, 0, 1)]], drain={0: lambda tz: p5_block(0, tz)})
    attention3(list(range(2, NB)),
               drain={0: lambda tz: out_proj(0, tz, (0, 1, 2)), 2: lambda tz: out_proj(0, tz, (3, 4)),
                      4: lambda tz: p5_block(1, tz)})

    def phase_g(u):
        p5_block(2 + u)
        out_proj(1 + u)
    rep(phase_g, NB - 2, 2)
    out_proj(NB - 1, split=True)

    def loop_f(i, carry):
        r0 = pl.multiple_of(i * 128, 128)
        pltpu.make_async_copy(oa_v.at[pl.ds(r0, 128), :], out_h.at[pl.ds(r0, 128), 0:D], osem.at[0, i]).wait()

        @pl.when(i < NB - 1)
        def _():
            pltpu.make_async_copy(ob_v.at[pl.ds(r0, 128), :], out_h.at[pl.ds(r0, 128), D:2 * D],
                                  osem.at[1, i]).wait()
        return carry
    jax.lax.fori_loop(0, NB, loop_f, 0)
    for n in range(5):
        last_copy(n).wait()


_CONSTS = _make_consts()


@jax.jit
def pallas_concat_heads__spectral_gfnet__sliding_block__prompt_kernel(A_x, A_w_r, A_w_i, B_x, B_wqkv, B_wo):
    mf, nf, g, hm = _CONSTS
    vm = pltpu.VMEM
    out = pl.pallas_call(
        _kernel,
        out_shape=jax.ShapeDtypeStruct((S, 2 * D), bf16),
        in_specs=[pl.BlockSpec(memory_space=pl.ANY)] * 10,
        out_specs=pl.BlockSpec(memory_space=pl.ANY),
        scratch_shapes=[
            vm((S, D), bf16), vm((DF, S), bf16), vm((DF, S), bf16), vm((S, D), bf16), vm((D, 3 * D), bf16),
            vm((D, D), bf16), vm((640, 256), bf16), vm((256, 640), bf16), vm((32, 128, 128), bf16),
            vm((32, 128, 128), bf16), vm((S, D), bf16), vm((S, D), bf16),
            vm((320, 256), u32), vm((128, 640), u32), vm((6, S, 128), f32), vm((4, 320, 128), f32),
            vm((6, 1024, 128), u32),
            vm((320, 1280), u32), vm((NB, 64, 640), u32), vm((320, 640), u32), vm((3, 128, 128), f32),
            vm((8, 128), i32), vm((NB, H, 16, 128), u32), vm((NB, H, 16, 128), u32), vm((NB, 64, 1024), u32),
            vm((NB, 64, 640), u32),
            pltpu.SemaphoreType.DMA((24,)), pltpu.SemaphoreType.DMA((2, NB)),
            pltpu.SemaphoreType.DMA((5,)),
        ],
        compiler_params=pltpu.CompilerParams(vmem_limit_bytes=120 * 1024 * 1024),
        name="fused_kernel",
    )(A_x.reshape(S, D), A_w_r.T, A_w_i.T, B_x.reshape(S, D), B_wqkv, B_wo, mf, nf, g, hm)
    return out.reshape(1, S, 2 * D)
```
